```python
import os as _os
_os.environ.setdefault("JAX_PLATFORMS", "cpu")
import jax
import jax.numpy as jnp

def _softmax(x, axis=-1):
    return jax.nn.softmax(x, axis=axis)
def _gelu(x):
    return jax.nn.gelu(x, approximate=True)
def _silu(x):
    return jax.nn.silu(x)
def _sigmoid(x):
    return jax.nn.sigmoid(x)
def _layernorm(x, axis=-1, eps=1e-5):
    m = jnp.mean(x, axis=axis, keepdims=True)
    v = jnp.var(x, axis=axis, keepdims=True)
    return (x - m) / jnp.sqrt(v + eps)
def _scatter_add(tgt, idx, src, axis=0):
    return tgt.at[idx].add(src)
def _segment_sum(src, seg, n):
    return jax.ops.segment_sum(src, seg, n)
class _Rng:
    def __init__(self, key):
        self._k = key
    def _next(self):
        self._k, sub = jax.random.split(self._k)
        return sub
    def normal(self, shape):
        return jax.random.normal(self._next(), shape, dtype=jnp.bfloat16)
    def randint(self, lo, hi, shape):
        return jax.random.randint(self._next(), shape, lo, hi, dtype=jnp.int32)
    def uniform(self, shape, lo=0.0, hi=1.0):
        return jax.random.uniform(self._next(), shape, jnp.bfloat16, lo, hi)
    def permutation(self, n):
        return jax.random.permutation(self._next(), n)


kernel_name = 'standalone__mha_softmax__prompt'

def setup_inputs():
    _rng = _Rng(jax.random.key(int.from_bytes(__import__("os").urandom(4), "little")))
    _w = (lambda a: (lambda t: t.astype(jnp.bfloat16) if jnp.issubdtype(t.dtype, jnp.floating) else t)(jnp.asarray(a)))
    B, H, Sq, Sk, D = 1, 32, 2048, 2048, 192
    return {
        "q": _w((lambda *s: _rng.normal(s) * 0.4)(B, H, Sq, D)),
        "k": _w((lambda *s: _rng.normal(s) * 0.4)(B, H, Sk, D)),
        "v": _w((lambda *s: _rng.normal(s) * 0.05)(B, H, Sk, D)),
    }

def reference(q, k, v):
    scale = q.shape[-1] ** -0.5
    scores = jnp.einsum("bhqd,bhkd->bhqk", q, k) * scale
    p = _softmax(scores, axis=-1)
    return jnp.einsum("bhqk,bhkd->bhqd", p, v)
```

```python
import functools, math
import jax, jax.numpy as jnp
from jax import lax
import jax.experimental.pallas as pl
import jax.experimental.pallas.tpu as pltpu

LOG2E = math.log2(math.e)
GW = 256

def t_kernel(qt_ref, kt_ref, vt_ref, ot_ref, k_scr, *s_scrs, scale, ck, pk, lead, fan, prescale, sum_mode):
    nb = len(s_scrs)
    D, Sq = qt_ref.shape
    Sk = kt_ref.shape[1]
    ng = Sq // GW
    c = scale * LOG2E
    cnt = [0]
    def zero(mult=8):
        cnt[0] += 1
        return pl.multiple_of(lax.shift_right_logical(pl.program_id(0) + cnt[0], 20), mult)
    k_scr[...] = pltpu.bitcast(kt_ref[...].T, jnp.uint32)

    mx = {}
    m_fin = {}
    def qk(g, i):
        qt = qt_ref[pl.ds(zero(16), D), g * GW:(g + 1) * GW]
        if prescale:
            qt = (qt.astype(jnp.float32) * c).astype(jnp.bfloat16)
        if g == 0:
            kk = k_scr[i * ck // 2:(i + 1) * ck // 2, :]
        else:
            kk = k_scr[pl.ds(zero() + i * ck // 2, ck // 2), :]
        kk = pltpu.bitcast(kk, jnp.bfloat16)
        st = jnp.dot(kk, qt, preferred_element_type=jnp.float32)
        s_scrs[g % nb][i * ck:(i + 1) * ck, :] = st
        accs = mx.get(g, [None] * fan)
        for r in range(ck // 8):
            x = st[r * 8:(r + 1) * 8]
            accs[r % fan] = x if accs[r % fan] is None else jnp.maximum(accs[r % fan], x)
        mx[g] = accs
        if (i + 1) * ck == Sk:
            while len(accs) > 1:
                accs = [jnp.maximum(accs[a], accs[a + 1]) for a in range(0, len(accs), 2)]
            m_fin[g] = jnp.max(accs[0], axis=0, keepdims=True)

    acc = {}
    lsum = {}
    zs = {}
    def pv(g, ct, kq):
        if g not in zs:
            zs[g] = zero()
        cs = slice(ct * 128, (ct + 1) * 128)
        s = s_scrs[g % nb][pl.ds(zs[g] + kq * pk, pk), cs]
        m = m_fin[g][:, cs]
        p = jnp.exp2(s - m) if prescale else jnp.exp2((s - m) * c)
        la = lsum.get((g, ct), [None] * 4)
        for t in range(pk // 128):
            for i in (range(7, -1, -1) if sum_mode == "desc" else range(8)):
                r = t * 128 + i * 16
                u = p[r:r + 8] + p[r + 8:r + 16]
                la[t % 4] = u if la[t % 4] is None else la[t % 4] + u
        lsum[(g, ct)] = la
        vv = vt_ref[pl.ds(zero(16), D), kq * pk:(kq + 1) * pk]
        o = jnp.dot(vv, p.astype(jnp.bfloat16), preferred_element_type=jnp.float32)
        acc[(g, ct)] = o if kq == 0 else acc[(g, ct)] + o
        if (kq + 1) * pk == Sk:
            l8 = (la[0] + la[1]) + (la[2] + la[3])
            l = jnp.sum(l8, axis=0, keepdims=True)
            col = g * GW + ct * 128
            ot_ref[:, col:col + 128] = (acc.pop((g, ct)) * (1.0 / l)).astype(ot_ref.dtype)

    qks = [(g, i) for g in range(ng) for i in range(Sk // ck)]
    pvs = [(g, ct, kq) for g in range(ng) for ct in range(GW // 128) for kq in range(Sk // pk)]
    qi = pi = 0
    qdone = 0
    pdone = 0
    while qi < len(qks) or pi < len(pvs):
        if qi < len(qks) and (qdone - pdone < Sk + lead or pi >= len(pvs)):
            qk(*qks[qi]); qi += 1; qdone += ck
        else:
            pv(*pvs[pi]); pi += 1; pdone += pk // 2

def attn_t(q, k, v, ck=256, pk=512, lead=1024, fan=2, prescale=True, sum_mode="desc", nb=None):
    B, H, Sq, D = q.shape
    Sk = k.shape[2]
    scale = D ** -0.5
    qt, kt, vt = (jnp.swapaxes(x, 2, 3) for x in (q, k, v))
    nb = nb or Sq // GW
    ot = pl.pallas_call(
        functools.partial(t_kernel, scale=scale, ck=ck, pk=pk, lead=lead, fan=fan, prescale=prescale, sum_mode=sum_mode),
        grid=(B * H,),
        in_specs=[
            pl.BlockSpec((None, None, D, Sq), lambda h: (0, h, 0, 0)),
            pl.BlockSpec((None, None, D, Sk), lambda h: (0, h, 0, 0)),
            pl.BlockSpec((None, None, D, Sk), lambda h: (0, h, 0, 0)),
        ],
        out_specs=pl.BlockSpec((None, None, D, Sq), lambda h: (0, h, 0, 0)),
        out_shape=jax.ShapeDtypeStruct(qt.shape, q.dtype),
        scratch_shapes=[pltpu.VMEM((Sk // 2, D), jnp.uint32)]
            + [pltpu.VMEM((Sk, GW), jnp.float32)] * nb,
        compiler_params=pltpu.CompilerParams(
            dimension_semantics=("parallel",),
            vmem_limit_bytes=100 * 1024 * 1024),
    )(qt, kt, vt)
    return jnp.swapaxes(ot, 2, 3)


@jax.jit
def pallas_standalone__mha_softmax__prompt_kernel(q: jax.Array, k: jax.Array, v: jax.Array):
    return attn_t(q, k, v)
```

```python
import functools, math
import jax, jax.numpy as jnp
from jax import lax
import jax.experimental.pallas as pl
import jax.experimental.pallas.tpu as pltpu

LOG2E = math.log2(math.e)
GW = 512
F32 = jnp.float32
BF16 = jnp.bfloat16
U32 = jnp.uint32

def emit(qk_groups, pv_groups, *, k_scr, s_scrs, v_scrs, q_scrs, p3_scrs, m_scr, vt_ref, ot_ref, c, cr, pk,
         aback, afrac, seed, D, Sk, r, lead, fwd, scale_in, skew3, out_hook=None, mid_hook=None):
    nb = len(s_scrs)
    T = D // 3
    cnt = [0]
    def zero(mult=8):
        cnt[0] += 1
        return pl.multiple_of(lax.shift_right_logical(seed + cnt[0], 20), mult)

    anchors = []
    mx = {}
    m_fin = {}
    staged_q = set()
    fwd_k = {}
    p3_of = {}
    p3_cnt = [0]
    done = {}
    wrows = {1: ((0, 2 * T),), 2: ((0, T), (2 * T, 3 * T)), 3: ((T, 3 * T),)}

    def prep_k(gi, i):
        kt_ref = qk_groups[gi][2]
        a = kt_ref[:, 2 * i * cr:(2 * i + 1) * cr]
        b = kt_ref[:, (2 * i + 1) * cr:(2 * i + 2) * cr]
        af, bf = a.astype(F32), b.astype(F32)
        if scale_in == "k":
            af, bf = af * c, bf * c
            a, b = af.astype(BF16), bf.astype(BF16)
        x = (af[T:2 * T] - b[T:2 * T].astype(F32)).astype(BF16)
        y = (bf[2 * T:] - a[2 * T:].astype(F32)).astype(BF16)
        l1 = jnp.concatenate([a[:T], x], axis=0).T
        l2 = jnp.concatenate([b[:T], y], axis=0).T
        l3 = jnp.concatenate([b[T:2 * T], a[2 * T:]], axis=0).T
        for w, l in ((1, l1), (2, l2), (3, l3)):
            k_scr[3 * i + w - 1][...] = pltpu.bitcast(l, U32)
            if fwd:
                fwd_k[(gi, i, w)] = l

    def qk(gi, i, w):
        g, qt_ref, kt_ref, carry = qk_groups[gi]
        qs = q_scrs[gi % len(q_scrs)]
        if gi not in staged_q:
            staged_q.add(gi)
            qt = qt_ref[:, g * GW:(g + 1) * GW]
            if scale_in == "q":
                qt = (qt.astype(F32) * c).astype(BF16)
            qs[...] = pltpu.bitcast(qt, U32)
            wt = jnp.concatenate([qt[lo:hi] for lo, hi in wrows[w]], axis=0)
        else:
            z = zero()
            wt = jnp.concatenate([pltpu.bitcast(qs[pl.ds(z + lo // 2, (hi - lo) // 2), :], BF16) for lo, hi in wrows[w]], axis=0)
        if kt_ref is not None and w == 3:
            prep_k(gi, i)
        if (gi, i, w) in fwd_k:
            kk = fwd_k.pop((gi, i, w))
        else:
            kk = pltpu.bitcast(k_scr[3 * i + w - 1][pl.ds(zero(), cr // 2), :], BF16)
        pw = jnp.dot(kk, wt, preferred_element_type=F32)
        ar = min(int(afrac * cr) // 8 * 8, cr - 8)
        anchors.append(pw[ar:ar + 8, :128])
        if w == 3:
            buf = p3_scrs[p3_cnt[0] % len(p3_scrs)]
            p3_cnt[0] += 1
            p3_of[(gi, i)] = buf
            buf[...] = pw
            return
        st = pw + p3_of[(gi, i)][pl.ds(zero(), cr), :]
        row = (2 * i + (w - 1)) * cr
        s_scrs[g % nb][row:row + cr, :] = st
        acc_m = mx.get(gi)
        for rr in range(cr // 8):
            x = st[rr * 8:(rr + 1) * 8]
            acc_m = x if acc_m is None else jnp.maximum(acc_m, x)
        mx[gi] = acc_m
        done[gi] = done.get(gi, 0) + cr
        if done[gi] == Sk:
            m = jnp.broadcast_to(jnp.max(acc_m, axis=0, keepdims=True), (8, GW))
            if carry:
                m_scr[g * 8:(g + 1) * 8, :] = m
            else:
                m_fin[g] = m

    acc = {}
    lsum = {}
    zs = {}
    def pv(g, ct, kq):
        if g not in zs:
            zs[g] = zero()
            if g < r:
                m_fin[g] = m_scr[g * 8:(g + 1) * 8, :]
        cs = slice(ct * 128, (ct + 1) * 128)
        s = s_scrs[g % nb][pl.ds(zs[g] + kq * pk, pk), cs]
        m = m_fin[g][:, cs]
        if aback and len(anchors) >= aback:
            a = anchors[-aback]
            m = jnp.where(a > jnp.inf, a, m)
        mb = jnp.concatenate([m] * (pk // 8), axis=0)
        p = jnp.exp2(s - mb) if scale_in != "none" else jnp.exp2((s - mb) * c)
        la = lsum.get((g, ct), [None] * 4)
        for t in range(pk // 128):
            for i in range(7, -1, -1):
                rr = t * 128 + i * 16
                u = p[rr:rr + 8] + p[rr + 8:rr + 16]
                la[t % 4] = u if la[t % 4] is None else la[t % 4] + u
        lsum[(g, ct)] = la
        if (g, ct) != (0, 0):
            vv = pltpu.bitcast(v_scrs[kq][pl.ds(zero(), D // 2), :], BF16)
        else:
            vv = vt_ref[:, kq * pk:(kq + 1) * pk]
            v_scrs[kq][...] = pltpu.bitcast(vv, U32)
        o = jnp.dot(vv, p.astype(BF16), preferred_element_type=F32)
        ar = min(int(afrac * D) // 8 * 8, D - 8)
        anchors.append(o[ar:ar + 8, :])
        acc[(g, ct)] = o if kq == 0 else acc[(g, ct)] + o
        if (kq + 1) * pk == Sk:
            l8 = (la[0] + la[1]) + (la[2] + la[3])
            l = jnp.sum(l8, axis=0, keepdims=True)
            col = g * GW + ct * 128
            ot_ref[:, col:col + 128] = (acc.pop((g, ct)) * (1.0 / l)).astype(ot_ref.dtype)
            if out_hook is not None:
                out_hook(col + 128)

    nch = Sk // (2 * cr)
    chunks = [(gi, i) for gi in range(len(qk_groups)) for i in range(nch)]
    qks = []
    if skew3:
        for n, ch in enumerate(chunks):
            if n == 0:
                qks.append(ch + (3,))
            if n + 1 < len(chunks):
                qks.append(chunks[n + 1] + (3,))
            qks.append(ch + (2,))
            qks.append(ch + (1,))
    else:
        qks = [ch + (w,) for ch in chunks for w in (3, 2, 1)]
    pvs = [(g, ct, kq) for g in pv_groups for ct in range(GW // 128) for kq in range(Sk // pk)]
    qi = pi = 0
    qt_, pt_ = 0, 0
    n = 0
    while qi < len(qks) or pi < len(pvs):
        if qi < len(qks) and (qt_ - pt_ < lead or pi >= len(pvs)):
            qk(*qks[qi]); qi += 1; qt_ += cr
        else:
            pv(*pvs[pi]); pi += 1; pt_ += D * pk // 512
        n += 1
        if mid_hook is not None:
            mid_hook(n)


def t_kernel(q_hbm, k_hbm, v_hbm, o_hbm, q_buf, k_buf, v_buf, o_buf, sem_in, sem_out, sem_fin, m_scr, *scrs,
             scale, cr, pk, aback, afrac, nb, nq, r, lead, fin_cols, dma_at, fwd, scale_in, skew3):
    H, D, Sq = q_hbm.shape[1:]
    Sk = k_hbm.shape[3]
    ng = Sq // GW
    nv = Sk // pk
    nk = 3 * Sk // (2 * cr)
    k_scr, scrs = scrs[:nk], scrs[nk:]
    s_scrs, v_scrs, q_scrs, p3_scrs = scrs[:nb], scrs[nb:nb + nv], scrs[nb + nv:nb + nv + nq], scrs[nb + nv + nq:]
    h = pl.program_id(0)
    slot = h % 2
    qa = r * GW
    def k_copy(hh, sl):
        return pltpu.make_async_copy(k_hbm.at[0, hh], k_buf.at[sl], sem_in.at[0, sl])
    def qa_copy(hh, sl):
        return pltpu.make_async_copy(q_hbm.at[0, hh, :, :qa], q_buf.at[sl, :, :qa], sem_in.at[1, sl])
    def qb_copy(hh, sl):
        return pltpu.make_async_copy(q_hbm.at[0, hh, :, qa:], q_buf.at[sl, :, qa:], sem_in.at[2, sl])
    def v_copy(hh, sl):
        return pltpu.make_async_copy(v_hbm.at[0, hh], v_buf.at[sl], sem_in.at[3, sl])
    def o_copy(hh, sl):
        return pltpu.make_async_copy(o_buf.at[sl], o_hbm.at[0, hh], sem_out.at[sl])
    edges = [0] + list(fin_cols) + [Sq]
    def o_fin(j):
        a, b = edges[j], edges[j + 1]
        sl = (H - 1) % 2
        return pltpu.make_async_copy(o_buf.at[sl, :, a:b], o_hbm.at[0, H - 1, :, a:b], sem_fin.at[j])

    common = dict(k_scr=k_scr, s_scrs=s_scrs, v_scrs=v_scrs, q_scrs=q_scrs, p3_scrs=p3_scrs, m_scr=m_scr,
                  c=scale * LOG2E, cr=cr, pk=pk, aback=aback, afrac=afrac, seed=h, D=D, Sk=Sk, r=r, lead=lead,
                  scale_in=scale_in, skew3=skew3)

    @pl.when(h == 0)
    def _():
        k_copy(0, 0).start()
        qa_copy(0, 0).start()
        v_copy(0, 0).start()
        qb_copy(0, 0).start()
        k_copy(1, 1).start()
        qa_copy(1, 1).start()
        k_copy(0, 0).wait()
        qa_copy(0, 0).wait()
        emit([(g, q_buf.at[0], k_buf.at[0] if g == 0 else None, True) for g in range(r)], [],
             vt_ref=None, ot_ref=None, fwd=fwd, **common)

    v_copy(h, slot).wait()
    qb_copy(h, slot).wait()
    @pl.when(h >= 2)
    def _():
        o_copy(h - 2, slot).wait()

    @pl.when(h < H - 1)
    def _():
        k_copy(h + 1, 1 - slot).wait()
        qa_copy(h + 1, 1 - slot).wait()
        def mid(n):
            if n == dma_at:
                v_copy(h + 1, 1 - slot).start()
                qb_copy(h + 1, 1 - slot).start()
                @pl.when(h + 2 < H)
                def _():
                    k_copy(h + 2, slot).start()
                    qa_copy(h + 2, slot).start()
        groups = ([(g, q_buf.at[slot], None, False) for g in range(r, ng)]
                  + [(g, q_buf.at[1 - slot], k_buf.at[1 - slot] if g == 0 else None, True) for g in range(r)])
        emit(groups, list(range(ng)), vt_ref=v_buf.at[slot], ot_ref=o_buf.at[slot], mid_hook=mid, fwd=False, **common)
        o_copy(h, slot).start()

    @pl.when(h == H - 1)
    def _():
        sl = (H - 1) % 2
        def out_hook(col):
            if col in edges[1:]:
                o_fin(edges.index(col) - 1).start()
        groups = [(g, q_buf.at[sl], None, False) for g in range(r, ng)]
        emit(groups, list(range(ng)), vt_ref=v_buf.at[sl], ot_ref=o_buf.at[sl], out_hook=out_hook, fwd=False, **common)
        o_copy(H - 2, 1 - sl).wait()
        for j in range(len(edges) - 1):
            o_fin(j).wait()


def attn_t(q, k, v, cr=128, pk=512, aback=5, afrac=1.0, nb=4, r=1, lead=768, fin_cols=(1536, 1920), dma_at=2,
           nq=2, fwd=False, scale_in="k", skew3=True, np3=3):
    B, H, Sq, D = q.shape
    Sk = k.shape[2]
    scale = D ** -0.5
    qt, kt, vt = (jnp.swapaxes(x, 2, 3) for x in (q, k, v))
    ot = pl.pallas_call(
        functools.partial(t_kernel, scale=scale, cr=cr, pk=pk, aback=aback, afrac=afrac, nb=nb, nq=nq, r=r,
                          lead=lead, fin_cols=fin_cols, dma_at=dma_at, fwd=fwd, scale_in=scale_in, skew3=skew3),
        grid=(H,),
        in_specs=[pl.BlockSpec(memory_space=pl.ANY)] * 3,
        out_specs=pl.BlockSpec(memory_space=pl.ANY),
        out_shape=jax.ShapeDtypeStruct(qt.shape, q.dtype),
        scratch_shapes=[pltpu.VMEM((2, D, Sq), BF16), pltpu.VMEM((2, D, Sk), BF16),
                        pltpu.VMEM((2, D, Sk), BF16), pltpu.VMEM((2, D, Sq), BF16),
                        pltpu.SemaphoreType.DMA((4, 2)), pltpu.SemaphoreType.DMA((2,)),
                        pltpu.SemaphoreType.DMA((len(fin_cols) + 1,)),
                        pltpu.VMEM((r * 8, GW), F32)]
            + [pltpu.VMEM((cr // 2, 2 * D // 3), U32)] * (3 * Sk // (2 * cr))
            + [pltpu.VMEM((Sk, GW), F32)] * nb
            + [pltpu.VMEM((D // 2, pk), U32)] * (Sk // pk)
            + [pltpu.VMEM((D // 2, GW), U32)] * nq
            + [pltpu.VMEM((cr, GW), F32)] * np3,
        compiler_params=pltpu.CompilerParams(
            dimension_semantics=("arbitrary",),
            vmem_limit_bytes=100 * 1024 * 1024, disable_bounds_checks=True),
    )(qt, kt, vt)
    return jnp.swapaxes(ot, 2, 3)


@jax.jit
def pallas_standalone__mha_softmax__prompt_kernel(q: jax.Array, k: jax.Array, v: jax.Array):
    return attn_t(q, k, v)
```

```python
import functools
import math

import jax
import jax.numpy as jnp
from jax import lax
import jax.experimental.pallas as pl
import jax.experimental.pallas.tpu as pltpu

F32 = jnp.float32
BF16 = jnp.bfloat16
U32 = jnp.uint32

GW = 512
CR = 128
PK = 512
PAD = 128
AHEAD = 2
N_S = 4
N_P3 = 4
LEAD = 384
ANCHOR = 740
DMA_AT = 4
K_FIRST = 4
LAST_EDGES = (1536, 1920)


def _emit(chunks, tail, pv_groups, groups, *, carried, fwd, skew, seed, vt_ref, ot_ref, hook,
          k_scr, s_scrs, v_scrs, q_scrs, p3_scrs, m_scr, c, D, Sk):
    T = D // 3
    cnt = [0]

    def zero():
        cnt[0] += 1
        if carried and cnt[0] <= 3:
            return 0
        return pl.multiple_of(lax.shift_right_logical(seed + cnt[0], 20), 8)

    anchors = []
    run_max = {}
    rows_done = {}
    m_fin = {}
    staged_q = set()
    fwd_k = {}
    p3_of = {}
    p3_cnt = [0]
    q_parts = {1: (0, 1), 2: (0, 2), 3: (1, 2)}
    if carried:
        staged_q.update({(chunks[0][0], j) for j in range(3)})
        p3_of[chunks[0]] = p3_scrs[0]
        p3_cnt[0] = 1

    def prep_k(gi, i):
        kt_ref = groups[gi][2]
        a = kt_ref[:, 2 * i * CR:(2 * i + 1) * CR]
        b = kt_ref[:, (2 * i + 1) * CR:(2 * i + 2) * CR]
        x = (a[T:2 * T].astype(F32) - b[T:2 * T].astype(F32)).astype(BF16)
        y = (b[2 * T:].astype(F32) - a[2 * T:].astype(F32)).astype(BF16)
        lhs = {1: jnp.concatenate([a[:T], x], axis=0).T,
               2: jnp.concatenate([b[:T], y], axis=0).T,
               3: jnp.concatenate([b[T:2 * T], a[2 * T:]], axis=0).T}
        for w, l in lhs.items():
            k_scr[3 * i + w - 1][...] = pltpu.bitcast(l, U32)
            if fwd:
                fwd_k[(gi, i, w)] = l

    def stage_q(gi, j):
        g, qt_ref = groups[gi][:2]
        staged_q.add((gi, j))
        qt = qt_ref[j * T:(j + 1) * T, g * GW:(g + 1) * GW]
        q_scrs[3 * (g % 2) + j][:, :GW] = pltpu.bitcast(qt, U32)
        return qt

    def qk(t, gi, i, w, p3_slot=None):
        g, _, kt_ref, carry = groups[gi]
        parts = []
        for j in q_parts[w]:
            if (gi, j) not in staged_q:
                parts.append(stage_q(gi, j))
            else:
                qs = q_scrs[3 * (g % 2) + j]
                parts.append(pltpu.bitcast(qs[pl.ds(zero(), T // 2), :GW], BF16))
        wt = jnp.concatenate(parts, axis=0)
        if kt_ref is not None and w == 3:
            prep_k(gi, i)
        if (gi, i, w) in fwd_k:
            kk = fwd_k.pop((gi, i, w))
        else:
            kk = pltpu.bitcast(k_scr[3 * i + w - 1][pl.ds(zero(), CR // 2), :], BF16)
        pw = jnp.dot(kk, wt, preferred_element_type=F32)
        anchors.append((t, CR, pw))
        if w == 3:
            if p3_slot is None:
                p3_slot = p3_cnt[0] % N_P3
                p3_cnt[0] += 1
            p3_of[(gi, i)] = p3_scrs[p3_slot]
            p3_scrs[p3_slot][:, :GW] = pw
            return
        st = (pw + p3_of[(gi, i)][pl.ds(zero(), CR), :GW]) * c
        row = (2 * i + (w - 1)) * CR
        s_scrs[g % N_S][row:row + CR, :GW] = st
        mx = run_max.get(gi)
        for rr in range(CR // 8):
            x = st[rr * 8:(rr + 1) * 8]
            mx = x if mx is None else jnp.maximum(mx, x)
        run_max[gi] = mx
        rows_done[gi] = rows_done.get(gi, 0) + CR
        if rows_done[gi] == Sk:
            m = jnp.broadcast_to(jnp.max(mx, axis=0, keepdims=True), (8, GW))
            if carry:
                m_scr[g * 8:(g + 1) * 8, :] = m
            else:
                m_fin[g] = m

    def pick_anchor(t):
        for (ts, rows, val) in reversed(anchors):
            if ts <= t - ANCHOR:
                rr = min((t - ANCHOR - ts) // 8 * 8, rows - 8)
                return val[rr:rr + 8, :128]
        return None

    acc = {}
    lsum = {}
    s_off = {}

    def pv(t, g, ct, kq):
        if g not in s_off:
            s_off[g] = zero()
            if g < AHEAD:
                m_fin[g] = m_scr[g * 8:(g + 1) * 8, :]
        cs = slice(ct * 128, (ct + 1) * 128)
        s = s_scrs[g % N_S][pl.ds(s_off[g] + kq * PK, PK), cs]
        m = m_fin[g][:, cs]
        a = pick_anchor(t)
        if a is not None:
            m = jnp.where(a > jnp.inf, a, m)
        p = jnp.exp2(s - jnp.concatenate([m] * (PK // 8), axis=0))
        la = lsum.get((g, ct), [None] * 4)
        for tt in range(PK // 128):
            for i in range(7, -1, -1):
                rr = tt * 128 + i * 16
                u = p[rr:rr + 8] + p[rr + 8:rr + 16]
                la[tt % 4] = u if la[tt % 4] is None else la[tt % 4] + u
        lsum[(g, ct)] = la
        if (g, ct) != (0, 0):
            vv = pltpu.bitcast(v_scrs[kq][pl.ds(zero(), D // 2), :PK], BF16)
        else:
            vv = vt_ref[:, kq * PK:(kq + 1) * PK]
            v_scrs[kq][:, :PK] = pltpu.bitcast(vv, U32)
        o = jnp.dot(vv, p.astype(BF16), preferred_element_type=F32)
        acc[(g, ct)] = o if kq == 0 else acc[(g, ct)] + o
        anchors.append((t, D, acc[(g, ct)]))
        if (kq + 1) * PK == Sk:
            l = jnp.sum((la[0] + la[1]) + (la[2] + la[3]), axis=0, keepdims=True)
            col = g * GW + ct * 128
            ot_ref[:, col:col + 128] = (acc.pop((g, ct)) * (1.0 / l)).astype(ot_ref.dtype)
            hook("out", col + 128)

    qks = []
    for n, ch in enumerate(chunks):
        if skew:
            if n == 0 and not carried:
                qks.append(ch + (3,))
            if n + 1 < len(chunks):
                qks.append(chunks[n + 1] + (3,))
        elif n > 0 or not carried:
            qks.append(ch + (3,))
        qks += [ch + (2,), ch + (1,)]
    pvs = [(g, ct, kq) for g in pv_groups for ct in range(GW // 128) for kq in range(Sk // PK)]

    qi = pi = 0
    tq = CR if carried else 0
    tp = 0
    while qi < len(qks) or pi < len(pvs):
        if qi < len(qks) and (tq - tp < LEAD or pi >= len(pvs)):
            hook("qk", qks[qi])
            qk(tq + tp, *qks[qi])
            qi += 1
            tq += CR
        else:
            pv(tq + tp, *pvs[pi])
            pi += 1
            tp += D * PK // 512
        hook("job", qi + pi)
    if tail is not None:
        stage_q(tail[0], 0)
        qk(tq + tp, *tail, 3, p3_slot=0)


def _kernel(q_hbm, k_hbm, v_hbm, o_hbm, in_buf, o_buf, sem_in, sem_pro, sem_out, m_scr, *scrs, c):
    H, D, Sq = q_hbm.shape
    Sk = k_hbm.shape[2]
    ng = Sq // GW
    nv = Sk // PK
    nch = Sk // (2 * CR)
    k_scr, scrs = scrs[:3 * nch], scrs[3 * nch:]
    s_scrs, scrs = scrs[:N_S], scrs[N_S:]
    v_scrs, scrs = scrs[:nv], scrs[nv:]
    q_scrs, p3_scrs = scrs[:6], scrs[6:]
    pid = pl.program_id(0)
    qa = (AHEAD + 1) * GW

    def start_inputs(h, hn, slot):
        pltpu.make_async_copy(v_hbm.at[h], in_buf.at[slot, 0], sem_in).start()
        pltpu.make_async_copy(q_hbm.at[h, :, qa:], in_buf.at[slot, 1, :, qa:], sem_in).start()
        pltpu.make_async_copy(k_hbm.at[hn], in_buf.at[slot, 2], sem_in).start()
        pltpu.make_async_copy(q_hbm.at[hn, :, :qa], in_buf.at[slot, 1, :, :qa], sem_in).start()

    def wait_inputs(slot):
        pltpu.make_async_copy(in_buf.at[slot], in_buf.at[slot], sem_in).wait()

    common = dict(k_scr=k_scr, s_scrs=s_scrs, v_scrs=v_scrs, q_scrs=q_scrs, p3_scrs=p3_scrs,
                  m_scr=m_scr, c=c, D=D, Sk=Sk)

    @pl.when(pid == 0)
    def _():
        ks = K_FIRST * 2 * CR
        first = [pltpu.make_async_copy(k_hbm.at[0, :, :ks], in_buf.at[1, 2, :, :ks], sem_pro.at[0]),
                 pltpu.make_async_copy(q_hbm.at[0, :, :GW], in_buf.at[1, 1, :, :GW], sem_pro.at[1])]
        second = [pltpu.make_async_copy(k_hbm.at[0, :, ks:], in_buf.at[1, 2, :, ks:], sem_pro.at[2]),
                  pltpu.make_async_copy(q_hbm.at[0, :, GW:qa], in_buf.at[1, 1, :, GW:qa], sem_pro.at[3])]
        for cp in first + second:
            cp.start()
        start_inputs(0, 1, 0)
        for cp in first:
            cp.wait()
        groups0 = [(g, in_buf.at[1, 1], in_buf.at[1, 2] if g == 0 else None, True)
                   for g in range(AHEAD + 1)]
        chunks0 = ([(g, i) for g in range(AHEAD) for i in range(K_FIRST)]
                   + [(g, i) for g in range(AHEAD) for i in range(K_FIRST, nch)])

        def hook0(kind, x):
            if kind == "qk" and x == chunks0[K_FIRST] + (3,):
                for cp in second:
                    cp.wait()

        _emit(chunks0, (AHEAD, 0), [], groups0, carried=False, fwd=True, skew=False, seed=pid,
              vt_ref=None, ot_ref=None, hook=hook0, **common)

        def body(h, carry):
            slot = lax.bitwise_and(h, 1)
            cur = in_buf.at[slot]
            wait_inputs(slot)

            def hook(kind, x):
                if kind == "job" and x == DMA_AT:
                    start_inputs(h + 1, jnp.minimum(h + 2, H - 1), 1 - slot)

            groups = ([(g, cur.at[1], None, False) for g in range(AHEAD, ng)]
                      + [(g, cur.at[1], cur.at[2] if g == 0 else None, True)
                         for g in range(AHEAD + 1)])
            chunks = [(gi, i) for gi in range(ng) for i in range(nch)]
            _emit(chunks, (ng, 0), list(range(ng)), groups, carried=True, fwd=False, skew=True,
                  seed=h, vt_ref=cur.at[0], ot_ref=o_buf.at[h], hook=hook, **common)
            pltpu.make_async_copy(o_buf.at[h], o_hbm.at[h], sem_out).start()
            return carry

        lax.fori_loop(0, H - 1, body, 0)

    @pl.when(pid == 1)
    def _():
        slot = (H - 1) % 2
        wait_inputs(slot)
        edges = [0, *LAST_EDGES, Sq]

        def hook(kind, col):
            if kind == "out" and col in edges[1:]:
                a = edges[edges.index(col) - 1]
                pltpu.make_async_copy(o_buf.at[H - 1, :, a:col], o_hbm.at[H - 1, :, a:col],
                                      sem_out).start()

        groups = [(g, in_buf.at[slot, 1], None, False) for g in range(AHEAD, ng)]
        chunks = [(gi, i) for gi in range(ng - AHEAD) for i in range(nch)]
        _emit(chunks, None, list(range(ng)), groups, carried=True, fwd=False, skew=True, seed=pid,
              vt_ref=in_buf.at[slot, 0], ot_ref=o_buf.at[H - 1], hook=hook, **common)
        pltpu.make_async_copy(o_buf, o_hbm, sem_out).wait()


@jax.jit
def pallas_standalone__mha_softmax__prompt_kernel(
    q: jax.Array,
    k: jax.Array,
    v: jax.Array,
):
    B, H, Sq, D = q.shape
    Sk = k.shape[2]
    BH = B * H
    assert D == 192 and Sq == Sk == N_S * GW and BH >= 2
    c = D ** -0.5 * math.log2(math.e)
    qt, kt, vt = (jnp.swapaxes(x, 2, 3).reshape(BH, D, Sq) for x in (q, k, v))
    scratch = (
        [pltpu.VMEM((2, 3, D, Sq), BF16),
         pltpu.VMEM((BH, D, Sq), BF16),
         pltpu.SemaphoreType.DMA(()),
         pltpu.SemaphoreType.DMA((4,)),
         pltpu.SemaphoreType.DMA(()),
         pltpu.VMEM((AHEAD * 8, GW), F32)]
        + [pltpu.VMEM((CR // 2, 2 * D // 3), U32)] * (3 * Sk // (2 * CR))
        + [pltpu.VMEM((Sk, GW + PAD), F32)] * N_S
        + [pltpu.VMEM((D // 2, PK + PAD), U32)] * (Sk // PK)
        + [pltpu.VMEM((D // 6, GW + PAD), U32)] * 6
        + [pltpu.VMEM((CR, GW + PAD), F32)] * N_P3
    )
    ot = pl.pallas_call(
        functools.partial(_kernel, c=c),
        grid=(2,),
        in_specs=[pl.BlockSpec(memory_space=pl.ANY)] * 3,
        out_specs=pl.BlockSpec(memory_space=pl.ANY),
        out_shape=jax.ShapeDtypeStruct((BH, D, Sq), q.dtype),
        scratch_shapes=scratch,
        compiler_params=pltpu.CompilerParams(
            dimension_semantics=("arbitrary",),
            vmem_limit_bytes=100 * 1024 * 1024,
            disable_bounds_checks=True,
        ),
    )(qt, kt, vt)
    return jnp.swapaxes(ot.reshape(B, H, D, Sq), 2, 3)
```

```python
import functools
import math

import jax
import jax.numpy as jnp
from jax import lax
import jax.experimental.pallas as pl
import jax.experimental.pallas.tpu as pltpu

F32 = jnp.float32
BF16 = jnp.bfloat16
U32 = jnp.uint32

GW = 512
CR = 128
NH = 2
PAD = 128
AHEAD = 2
N_S = 4
N_P3 = 4
N_SUM = 8
A_ORDER = (5, 3, 2, 4)
B_ORDER = (1, 7, 6)
A_TIE = 440
B_TIE = 400
MAIN_ORDER = ("Q" + "QQA" * 8, "QQA" * 2 + "QBA" * 6)
LAST_ORDER = ("QQA" * 8, "QQA" * 2 + "QBA" * 6)
DMA_AT = 4
K_FIRST = 4
LAST_EDGES = (1536, 1792)


def _emit(chunks, tail, pv_groups, groups, *, order, carried, fwd, skew, seed, vt_ref, ot_ref, hook,
          k_scr, s_scrs, a_scrs, q_scrs, p3_scrs, r_scrs, p_scrs, m_scr, c, D, Sk):
    T = D // 3
    Dh = D // 2
    R = Sk // 2 // NH
    cnt = [0]

    def zero():
        cnt[0] += 1
        if carried and cnt[0] <= 3:
            return 0
        return pl.multiple_of(lax.shift_right_logical(seed + cnt[0], 20), 8)

    def rep(x, rows):
        return jnp.concatenate([x] * (rows // 8), axis=0)

    results = []

    def tie(x, t, dist):
        for (ts, rows, val) in reversed(results):
            if ts <= t - dist:
                rr = min((t - dist - ts) // 8 * 8, rows - 8)
                a = val[rr:rr + 8, :128]
                return jnp.where(a > jnp.inf, a, x)
        return x

    run_max = {}
    rows_done = {}
    m_fin = {}
    staged_q = set()
    fwd_k = {}
    p3_of = {}
    p3_cnt = [0]
    q_parts = {1: (0, 1), 2: (0, 2), 3: (1, 2)}
    if carried:
        staged_q.update({(chunks[0][0], j) for j in range(3)})
        p3_of[chunks[0]] = p3_scrs[0]
        p3_cnt[0] = 1

    def prep_k(gi, i):
        kt_ref = groups[gi][2]
        a = kt_ref[:, 2 * i * CR:(2 * i + 1) * CR]
        b = kt_ref[:, (2 * i + 1) * CR:(2 * i + 2) * CR]
        x = (a[T:2 * T].astype(F32) - b[T:2 * T].astype(F32)).astype(BF16)
        y = (b[2 * T:].astype(F32) - a[2 * T:].astype(F32)).astype(BF16)
        lhs = {1: jnp.concatenate([a[:T], x], axis=0).T,
               2: jnp.concatenate([b[:T], y], axis=0).T,
               3: jnp.concatenate([b[T:2 * T], a[2 * T:]], axis=0).T}
        for w, l in lhs.items():
            k_scr[3 * i + w - 1][...] = pltpu.bitcast(l, U32)
            if fwd:
                fwd_k[(gi, i, w)] = l

    def stage_q(gi, j):
        g, qt_ref = groups[gi][:2]
        staged_q.add((gi, j))
        qt = qt_ref[j * T:(j + 1) * T, g * GW:(g + 1) * GW]
        q_scrs[3 * (g % 2) + j][:, :GW] = pltpu.bitcast(qt, U32)
        return qt

    def qk(t, gi, i, w, p3_slot=None):
        g, _, kt_ref, carry = groups[gi]
        parts = []
        for j in q_parts[w]:
            if (gi, j) not in staged_q:
                parts.append(stage_q(gi, j))
            else:
                qs = q_scrs[3 * (g % 2) + j]
                parts.append(pltpu.bitcast(qs[pl.ds(zero(), T // 2), :GW], BF16))
        wt = jnp.concatenate(parts, axis=0)
        if kt_ref is not None and w == 3:
            prep_k(gi, i)
        if (gi, i, w) in fwd_k:
            kk = fwd_k.pop((gi, i, w))
        else:
            kk = pltpu.bitcast(k_scr[3 * i + w - 1][pl.ds(zero(), CR // 2), :], BF16)
        pw = jnp.dot(kk, wt, preferred_element_type=F32)
        results.append((t, CR, pw))
        if w == 3:
            if p3_slot is None:
                p3_slot = p3_cnt[0] % N_P3
                p3_cnt[0] += 1
            p3_of[(gi, i)] = p3_scrs[p3_slot]
            p3_scrs[p3_slot][:, :GW] = pw
            return
        st = (pw + p3_of[(gi, i)][pl.ds(zero(), CR), :GW]) * c
        row = (w - 1) * (Sk // 2) + i * CR
        s_scrs[g % N_S][row:row + CR, :GW] = st
        mx = run_max.get(gi)
        for rr in range(CR // 8):
            x = st[rr * 8:(rr + 1) * 8]
            mx = x if mx is None else jnp.maximum(mx, x)
        run_max[gi] = mx
        rows_done[gi] = rows_done.get(gi, 0) + CR
        if rows_done[gi] == Sk:
            m = jnp.broadcast_to(jnp.max(mx, axis=0, keepdims=True), (8, GW))
            if carry:
                m_scr[g * 8:(g + 1) * 8, :] = m
            else:
                m_fin[g] = m

    s_off = {}
    state = {}

    def a_operand(i, hf):
        tiles = []
        for kp in range(hf * R // 128, (hf + 1) * R // 128):
            def blk(r, kr):
                return vt_ref[r * Dh:(r + 1) * Dh, (2 * kp + kr) * 128:(2 * kp + kr + 1) * 128]

            def add(x, y):
                return (blk(*x).astype(F32) + blk(*y).astype(F32)).astype(BF16)

            def sub(x, y):
                return (blk(*x).astype(F32) - blk(*y).astype(F32)).astype(BF16)

            tiles.append({1: lambda: add((0, 0), (1, 1)), 2: lambda: add((1, 0), (1, 1)),
                          3: lambda: blk(0, 0), 4: lambda: blk(1, 1),
                          5: lambda: add((0, 0), (0, 1)), 6: lambda: sub((1, 0), (0, 0)),
                          7: lambda: sub((0, 1), (1, 1))}[i]())
        return jnp.concatenate(tiles, axis=1)

    def pv(t, g, u, i, hf):
        if g not in s_off:
            s_off[g] = zero()
            if g < AHEAD:
                m_fin[g] = m_scr[g * 8:(g + 1) * 8, :]
        st = state.setdefault((g, u), {})

        def pbuf(kr, cx):
            return p_scrs[(u * 4 + kr * 2 + cx) * NH + hf]

        def fresh(kr, cx):
            cs = slice((2 * u + cx) * 128, (2 * u + cx + 1) * 128)
            s = s_scrs[g % N_S][pl.ds(s_off[g] + kr * (Sk // 2) + hf * R, R), cs]
            p = jnp.exp2(s - rep(tie(m_fin[g][:, cs], t, A_TIE), R))
            pbuf(kr, cx)[...] = p
            return p

        def load(kr, cx):
            return pbuf(kr, cx)[pl.ds(zero(), R), :]

        def eager_sum(cx, p):
            la = st.get(("l", cx), [None] * 4)
            for tt in range(R // 128):
                for ii in range(7, -1, -1):
                    rr = tt * 128 + ii * 16
                    v = p[rr:rr + 8] + p[rr + 8:rr + 16]
                    la[tt % 4] = v if la[tt % 4] is None else la[tt % 4] + v
            if hf + 1 == NH:
                la = [(la[0] + la[1]) + (la[2] + la[3])] + [None] * (N_SUM - 1)
            st[("l", cx)] = la

        def lazy_sum(kr, cx):
            x = load(kr, cx)
            la = st[("l", cx)]
            for rr in range(R // 8):
                v = x[rr * 8:(rr + 1) * 8]
                la[rr % N_SUM] = v if la[rr % N_SUM] is None else la[rr % N_SUM] + v

        def total(cx):
            l8 = functools.reduce(lambda a, b: a + b, st[("l", cx)])
            return jnp.broadcast_to(jnp.sum(l8, axis=0, keepdims=True), (8, 128))

        def cross(kx, ky):
            if "rho" not in st:
                lx = total(0)
                st["rx"] = 1.0 / lx
                st["ry"] = 1.0 / total(1)
                st["rho"] = lx * st["ry"]
            rho = tie(st["rho"], t, B_TIE)
            return load(kx, 0) - rep(rho, R) * load(ky, 1)

        if i == 2:
            w = fresh(0, 0)
            eager_sum(0, w)
        elif i == 4:
            w = fresh(1, 0) - load(0, 0)
            lazy_sum(1, 0)
        elif i == 5:
            w = fresh(1, 1)
            eager_sum(1, w)
        elif i == 3:
            w = load(1, 1) - fresh(0, 1)
            lazy_sum(0, 1)
        else:
            w = cross(*{1: (0, 1), 6: (0, 0), 7: (1, 1)}[i])
        if (g, u) != (0, 0):
            av = pltpu.bitcast(a_scrs[(i - 1) * NH + hf][pl.ds(zero(), Dh // 2), :], BF16)
        else:
            av = a_operand(i, hf)
            a_scrs[(i - 1) * NH + hf][...] = pltpu.bitcast(av, U32)
        mi = jnp.dot(av, w.astype(BF16), preferred_element_type=F32)
        if hf > 0:
            mi = mi + st.pop(("part", i))
        results.append((t, Dh, mi))
        if hf + 1 < NH:
            st[("part", i)] = mi
            return
        col = g * GW + u * 256

        def out(r, cx, x, scale):
            ot_ref[r * Dh:(r + 1) * Dh, col + cx * 128:col + (cx + 1) * 128] = (
                x * rep(scale, Dh)).astype(ot_ref.dtype)

        if i in A_ORDER:
            r_scrs[u * 4 + i - 2][...] = mi
        elif i == 1:
            m2, m3, m4, m5 = (r_scrs[u * 4 + j][pl.ds(zero(), Dh), :] for j in range(4))
            out(1, 0, m2 + m4, st["rx"])
            out(0, 1, m5 - m3, st["ry"])
            st["c11"] = mi + (m4 + rep(st["rho"], Dh) * m5)
            st["c22"] = (m2 - rep(st["rho"], Dh) * m3) - mi
        elif i == 6:
            out(1, 1, st.pop("c22") - mi, st["rx"])
        else:
            out(0, 0, mi + st.pop("c11"), st["rx"])
        if i == B_ORDER[-1]:
            hook("out", col + 256)

    q_jobs = []
    for n, ch in enumerate(chunks):
        if skew:
            if n == 0 and not carried:
                q_jobs.append(ch + (3,))
            if n + 1 < len(chunks):
                q_jobs.append(chunks[n + 1] + (3,))
        elif n > 0 or not carried:
            q_jobs.append(ch + (3,))
        q_jobs += [ch + (2,), ch + (1,)]
    pairs = [(g, u) for g in pv_groups for u in range(2)]
    a_jobs = [pr + (i, hf) for pr in pairs for i in A_ORDER for hf in range(NH)]
    b_jobs = [pr + (i, hf) for pr in pairs for i in B_ORDER for hf in range(NH)]
    na, nb = len(A_ORDER) * NH, len(B_ORDER) * NH
    prefix, cycle = order
    qi = ai = bi = pos = t = 0
    while qi < len(q_jobs) or ai < len(a_jobs) or bi < len(b_jobs):
        tok = prefix[pos] if pos < len(prefix) else cycle[(pos - len(prefix)) % len(cycle)]
        pos += 1
        if tok == "Q":
            if qi >= len(q_jobs):
                continue
            g, _, _, carry = groups[q_jobs[qi][0]]
            assert not (carry and a_jobs) or ai >= 2 * na * (g + 1)
            hook("qk", q_jobs[qi])
            qk(t, *q_jobs[qi])
            qi += 1
            t += CR
        elif tok == "A":
            if ai >= len(a_jobs):
                continue
            assert ai // na - bi // nb < 2
            pv(t, *a_jobs[ai])
            ai += 1
            t += Dh
        else:
            if bi >= len(b_jobs) or ai < min((bi // nb + 1) * na + 1, len(a_jobs)):
                continue
            pv(t, *b_jobs[bi])
            bi += 1
            t += Dh
        hook("job", qi + ai + bi)
    if tail is not None:
        stage_q(tail[0], 0)
        qk(t, *tail, 3, p3_slot=0)


def _kernel(q_hbm, k_hbm, v_hbm, o_hbm, in_buf, o_buf, sem_in, sem_pro, sem_out, m_scr, *scrs, c):
    H, D, Sq = q_hbm.shape
    Sk = k_hbm.shape[2]
    ng = Sq // GW
    nch = Sk // (2 * CR)
    k_scr, scrs = scrs[:3 * nch], scrs[3 * nch:]
    s_scrs, scrs = scrs[:N_S], scrs[N_S:]
    a_scrs, scrs = scrs[:7 * NH], scrs[7 * NH:]
    q_scrs, scrs = scrs[:6], scrs[6:]
    p3_scrs, scrs = scrs[:N_P3], scrs[N_P3:]
    r_scrs, p_scrs = scrs[:8], scrs[8:]
    pid = pl.program_id(0)
    qa = (AHEAD + 1) * GW

    def start_inputs(h, hn, slot):
        pltpu.make_async_copy(v_hbm.at[h], in_buf.at[slot, 0], sem_in).start()
        pltpu.make_async_copy(q_hbm.at[h, :, qa:], in_buf.at[slot, 1, :, qa:], sem_in).start()
        pltpu.make_async_copy(k_hbm.at[hn], in_buf.at[slot, 2], sem_in).start()
        pltpu.make_async_copy(q_hbm.at[hn, :, :qa], in_buf.at[slot, 1, :, :qa], sem_in).start()

    def wait_inputs(slot):
        pltpu.make_async_copy(in_buf.at[slot], in_buf.at[slot], sem_in).wait()

    common = dict(k_scr=k_scr, s_scrs=s_scrs, a_scrs=a_scrs, q_scrs=q_scrs, p3_scrs=p3_scrs,
                  r_scrs=r_scrs, p_scrs=p_scrs, m_scr=m_scr, c=c, D=D, Sk=Sk)

    @pl.when(pid == 0)
    def _():
        ks = K_FIRST * 2 * CR
        first = [pltpu.make_async_copy(k_hbm.at[0, :, :ks], in_buf.at[1, 2, :, :ks], sem_pro.at[0]),
                 pltpu.make_async_copy(q_hbm.at[0, :, :GW], in_buf.at[1, 1, :, :GW], sem_pro.at[1])]
        second = [pltpu.make_async_copy(k_hbm.at[0, :, ks:], in_buf.at[1, 2, :, ks:], sem_pro.at[2]),
                  pltpu.make_async_copy(q_hbm.at[0, :, GW:qa], in_buf.at[1, 1, :, GW:qa], sem_pro.at[3])]
        for cp in first + second:
            cp.start()
        start_inputs(0, 1, 0)
        for cp in first:
            cp.wait()
        groups0 = [(g, in_buf.at[1, 1], in_buf.at[1, 2] if g == 0 else None, True)
                   for g in range(AHEAD + 1)]
        chunks0 = ([(g, i) for g in range(AHEAD) for i in range(K_FIRST)]
                   + [(g, i) for g in range(AHEAD) for i in range(K_FIRST, nch)])

        def hook0(kind, x):
            if kind == "qk" and x == chunks0[K_FIRST] + (3,):
                for cp in second:
                    cp.wait()

        _emit(chunks0, (AHEAD, 0), [], groups0, order=("", "Q"), carried=False, fwd=True, skew=False,
              seed=pid, vt_ref=None, ot_ref=None, hook=hook0, **common)

        def body(h, carry):
            slot = lax.bitwise_and(h, 1)
            cur = in_buf.at[slot]
            wait_inputs(slot)

            def hook(kind, x):
                if kind == "job" and x == DMA_AT:
                    start_inputs(h + 1, jnp.minimum(h + 2, H - 1), 1 - slot)

            groups = ([(g, cur.at[1], None, False) for g in range(AHEAD, ng)]
                      + [(g, cur.at[1], cur.at[2] if g == 0 else None, True)
                         for g in range(AHEAD + 1)])
            chunks = [(gi, i) for gi in range(ng) for i in range(nch)]
            _emit(chunks, (ng, 0), list(range(ng)), groups, order=MAIN_ORDER, carried=True,
                  fwd=False, skew=True, seed=h, vt_ref=cur.at[0], ot_ref=o_buf.at[h], hook=hook,
                  **common)
            pltpu.make_async_copy(o_buf.at[h], o_hbm.at[h], sem_out).start()
            return carry

        lax.fori_loop(0, H - 1, body, 0)

    @pl.when(pid == 1)
    def _():
        slot = (H - 1) % 2
        wait_inputs(slot)
        edges = [0, *LAST_EDGES, Sq]

        def hook(kind, col):
            if kind == "out" and col in edges[1:]:
                a = edges[edges.index(col) - 1]
                pltpu.make_async_copy(o_buf.at[H - 1, :, a:col], o_hbm.at[H - 1, :, a:col],
                                      sem_out).start()

        groups = [(g, in_buf.at[slot, 1], None, False) for g in range(AHEAD, ng)]
        chunks = [(gi, i) for gi in range(ng - AHEAD) for i in range(nch)]
        _emit(chunks, None, list(range(ng)), groups, order=LAST_ORDER, carried=True, fwd=False,
              skew=True, seed=pid, vt_ref=in_buf.at[slot, 0], ot_ref=o_buf.at[H - 1], hook=hook,
              **common)
        pltpu.make_async_copy(o_buf, o_hbm, sem_out).wait()


@jax.jit
def pallas_standalone__mha_softmax__prompt_kernel(
    q: jax.Array,
    k: jax.Array,
    v: jax.Array,
):
    B, H, Sq, D = q.shape
    Sk = k.shape[2]
    BH = B * H
    assert D == 192 and Sq == Sk == N_S * GW and BH >= 2
    c = D ** -0.5 * math.log2(math.e)
    R = Sk // 2 // NH
    qt, kt, vt = (jnp.swapaxes(x, 2, 3).reshape(BH, D, Sq) for x in (q, k, v))
    scratch = (
        [pltpu.VMEM((2, 3, D, Sq), BF16),
         pltpu.VMEM((BH, D, Sq), BF16),
         pltpu.SemaphoreType.DMA(()),
         pltpu.SemaphoreType.DMA((4,)),
         pltpu.SemaphoreType.DMA(()),
         pltpu.VMEM((AHEAD * 8, GW), F32)]
        + [pltpu.VMEM((CR // 2, 2 * D // 3), U32)] * (3 * Sk // (2 * CR))
        + [pltpu.VMEM((Sk, GW + PAD), F32)] * N_S
        + [pltpu.VMEM((D // 4, R), U32)] * (7 * NH)
        + [pltpu.VMEM((D // 6, GW + PAD), U32)] * 6
        + [pltpu.VMEM((CR, GW + PAD), F32)] * N_P3
        + [pltpu.VMEM((D // 2, 128), F32)] * 8
        + [pltpu.VMEM((R, 128), F32)] * (8 * NH)
    )
    ot = pl.pallas_call(
        functools.partial(_kernel, c=c),
        grid=(2,),
        in_specs=[pl.BlockSpec(memory_space=pl.ANY)] * 3,
        out_specs=pl.BlockSpec(memory_space=pl.ANY),
        out_shape=jax.ShapeDtypeStruct((BH, D, Sq), q.dtype),
        scratch_shapes=scratch,
        compiler_params=pltpu.CompilerParams(
            dimension_semantics=("arbitrary",),
            vmem_limit_bytes=100 * 1024 * 1024,
            disable_bounds_checks=True,
        ),
    )(qt, kt, vt)
    return jnp.swapaxes(ot.reshape(B, H, D, Sq), 2, 3)
```

```python
import functools
import math

import jax
import jax.numpy as jnp
from jax import lax
import jax.experimental.pallas as pl
import jax.experimental.pallas.tpu as pltpu

F32 = jnp.float32
BF16 = jnp.bfloat16
U32 = jnp.uint32

GW = 512
CR = 128
NH = 2
PAD = 128
AHEAD = 2
N_S = 4
N_P3 = 2
N_SUM = 6
B_ORDER = (1, 6, 7)
MAIN_PLAN = ("QA" + "QQA" * 7, "QQAQBAQQA" + "QBA" * 5, (5, 2, 4, 3), 258, 298)
LAST_PLAN = ("QQA" * 8, "QQA" * 2 + "QBA" * 6, (5, 3, 2, 4), 234, 242)
DMA_AT = 40
K_FIRST = 4
LAST_EDGES = (1536, 1792)


def _emit(chunks, tail, pv_groups, groups, *, plan, carried, fwd, seed, vt_ref, ot_ref, hook,
          k_scr, s_scrs, a_scrs, q_scrs, p3_scrs, p3_wide, r_scrs, p_scrs, m_scr, c, D, Sk):
    T = D // 3
    Dh = D // 2
    R = Sk // 2 // NH
    prefix, cycle, a_order, a_tie, b_tie = plan
    cnt = [0]

    def zero():
        cnt[0] += 1
        if carried and cnt[0] <= 3:
            return 0
        return pl.multiple_of(lax.shift_right_logical(seed + cnt[0], 20), 8)

    def rep(x, rows):
        return jnp.concatenate([x] * (rows // 8), axis=0)

    starts = []
    results = []

    def tie(x, dist):
        t = starts[-3] if len(starts) >= 3 else starts[-1]
        for (ts, rows, val) in reversed(results):
            if ts <= t - dist:
                rr = min((t - dist - ts) // 8 * 8, rows - 8)
                a = val[rr:rr + 8, :128]
                return jnp.where(a > jnp.inf, a, x)
        return x

    run_max = {}
    tiles_done = {}
    m_fin = {}
    staged_q = set()
    fwd_k = {}
    q_parts = {1: (0, 1), 2: (0, 2), 3: (1, 2)}
    if carried:
        staged_q.update({(chunks[0][0], j) for j in range(3)})

    def prep_k(gi, i):
        kt_ref = groups[gi][2]
        a = kt_ref[:, 2 * i * CR:(2 * i + 1) * CR]
        b = kt_ref[:, (2 * i + 1) * CR:(2 * i + 2) * CR]
        x = (a[T:2 * T].astype(F32) - b[T:2 * T].astype(F32)).astype(BF16)
        y = (b[2 * T:].astype(F32) - a[2 * T:].astype(F32)).astype(BF16)
        lhs = {1: jnp.concatenate([a[:T], x], axis=0).T,
               2: jnp.concatenate([b[:T], y], axis=0).T,
               3: jnp.concatenate([b[T:2 * T], a[2 * T:]], axis=0).T}
        for w, l in lhs.items():
            k_scr[3 * i + w - 1][...] = pltpu.bitcast(l, U32)
            if fwd:
                fwd_k[(gi, i, w)] = l

    def stage_q(gi, j):
        g, qt_ref = groups[gi][:2]
        staged_q.add((gi, j))
        qt = qt_ref[j * T:(j + 1) * T, g * GW:(g + 1) * GW]
        q_scrs[3 * (g % 2) + j][:, :GW] = pltpu.bitcast(qt, U32)
        return qt

    def q_third(gi, j):
        if (gi, j) not in staged_q:
            return stage_q(gi, j)
        qs = q_scrs[3 * (groups[gi][0] % 2) + j]
        return pltpu.bitcast(qs[pl.ds(zero(), T // 2), :GW], BF16)

    def k_operand(gi, i, w):
        if (gi, i, w) in fwd_k:
            return fwd_k.pop((gi, i, w))
        return pltpu.bitcast(k_scr[3 * i + w - 1][pl.ds(zero(), CR // 2), :], BF16)

    def finish(gi, i, w, ct, s):
        g, _, _, carry = groups[gi]
        s = s * c
        row = (w - 1) * (Sk // 2) + i * CR
        s_scrs[g % N_S][row:row + CR, ct * 128:ct * 128 + s.shape[1]] = s
        for n in range(s.shape[1] // 128):
            mx = run_max.get((gi, ct + n))
            for rr in range(CR // 8):
                x = s[rr * 8:(rr + 1) * 8, n * 128:(n + 1) * 128]
                mx = x if mx is None else jnp.maximum(mx, x)
            run_max[(gi, ct + n)] = mx
        tiles_done[gi] = tiles_done.get(gi, 0) + s.shape[1] // 128
        if tiles_done[gi] == (Sk // CR) * (GW // 128):
            mx = jnp.concatenate([run_max[(gi, n)] for n in range(GW // 128)], axis=1)
            m = jnp.broadcast_to(jnp.max(mx, axis=0, keepdims=True), (8, GW))
            if carry:
                m_scr[g * 8:(g + 1) * 8, :] = m
            else:
                m_fin[g] = m

    def qk_pass(gi, i, w):
        wt = jnp.concatenate([q_third(gi, j) for j in q_parts[w]], axis=0)
        pw = jnp.dot(k_operand(gi, i, w), wt, preferred_element_type=F32)
        results.append((starts[-1], CR, pw))
        if w == 3:
            p3_wide[:, :GW] = pw
        else:
            finish(gi, i, w, 0, pw + p3_wide[pl.ds(zero(), CR), :GW])

    def qk_round(gi, i, rnd):
        qv = [q_third(gi, j) for j in range(3)]
        if groups[gi][2] is not None and rnd == 0:
            prep_k(gi, i)
        kk = {w: k_operand(gi, i, w) for w in (1, 2, 3)}

        def dot(w, ct):
            wt = jnp.concatenate([qv[j][:, ct * 128:(ct + 1) * 128] for j in q_parts[w]], axis=0)
            return jnp.dot(kk[w], wt, preferred_element_type=F32)

        p3 = dot(3, rnd)
        results.append((starts[-1], CR, p3))
        finish(gi, i, 1, rnd, dot(1, rnd) + p3)
        finish(gi, i, 2, rnd, dot(2, rnd) + p3)
        if rnd == 0:
            p3_scrs[i % N_P3][...] = dot(3, 3)
        else:
            finish(gi, i, rnd, 3, dot(rnd, 3) + p3_scrs[i % N_P3][pl.ds(zero(), CR), :])

    s_off = {}
    state = {}

    def a_operand(i, hf):
        tiles = []
        for kp in range(hf * R // 128, (hf + 1) * R // 128):
            def blk(r, kr):
                return vt_ref[r * Dh:(r + 1) * Dh, (2 * kp + kr) * 128:(2 * kp + kr + 1) * 128]

            def add(x, y):
                return (blk(*x).astype(F32) + blk(*y).astype(F32)).astype(BF16)

            def sub(x, y):
                return (blk(*x).astype(F32) - blk(*y).astype(F32)).astype(BF16)

            tiles.append({1: lambda: add((0, 0), (1, 1)), 2: lambda: add((1, 0), (1, 1)),
                          3: lambda: blk(0, 0), 4: lambda: blk(1, 1),
                          5: lambda: add((0, 0), (0, 1)), 6: lambda: sub((1, 0), (0, 0)),
                          7: lambda: sub((0, 1), (1, 1))}[i]())
        return jnp.concatenate(tiles, axis=1)

    def pv(g, u, i, hf):
        if g not in s_off:
            s_off[g] = zero()
            if g < AHEAD:
                m_fin[g] = m_scr[g * 8:(g + 1) * 8, :]
        st = state.setdefault((g, u), {})

        def pbuf(kr, cx):
            return p_scrs[(u * 4 + kr * 2 + cx) * NH + hf]

        def fresh(kr, cx):
            cs = slice((2 * u + cx) * 128, (2 * u + cx + 1) * 128)
            s = s_scrs[g % N_S][pl.ds(s_off[g] + kr * (Sk // 2) + hf * R, R), cs]
            p = jnp.exp2(s - rep(tie(m_fin[g][:, cs], a_tie), R))
            pbuf(kr, cx)[...] = p
            return p

        def load(kr, cx):
            return pbuf(kr, cx)[pl.ds(zero(), R), :]

        def eager_sum(cx, p):
            la = st.get(("l", cx), [None] * 4)
            for tt in range(R // 128):
                for ii in range(7, -1, -1):
                    rr = tt * 128 + ii * 16
                    v = p[rr:rr + 8] + p[rr + 8:rr + 16]
                    la[tt % 4] = v if la[tt % 4] is None else la[tt % 4] + v
            if hf + 1 == NH:
                la = [(la[0] + la[1]) + (la[2] + la[3])] + [None] * (N_SUM - 1)
            st[("l", cx)] = la

        def lazy_sum(kr, cx):
            x = load(kr, cx)
            la = st[("l", cx)]
            for rr in range(R // 8):
                v = x[rr * 8:(rr + 1) * 8]
                la[rr % N_SUM] = v if la[rr % N_SUM] is None else la[rr % N_SUM] + v

        def total(cx):
            l8 = functools.reduce(lambda a, b: a + b, st[("l", cx)])
            return jnp.broadcast_to(jnp.sum(l8, axis=0, keepdims=True), (8, 128))

        def cross(kx, ky):
            if "rho" not in st:
                lx = total(0)
                st["rx"] = 1.0 / lx
                st["ry"] = 1.0 / total(1)
                st["rho"] = lx * st["ry"]
            rho = tie(st["rho"], b_tie)
            return load(kx, 0) - rep(rho, R) * load(ky, 1)

        if i == 2:
            w = fresh(0, 0)
            eager_sum(0, w)
        elif i == 4:
            w = fresh(1, 0) - load(0, 0)
            lazy_sum(1, 0)
        elif i == 5:
            w = fresh(1, 1)
            eager_sum(1, w)
        elif i == 3:
            w = load(1, 1) - fresh(0, 1)
            lazy_sum(0, 1)
        else:
            w = cross(*{1: (0, 1), 6: (0, 0), 7: (1, 1)}[i])
        if (g, u) != (0, 0):
            av = pltpu.bitcast(a_scrs[(i - 1) * NH + hf][pl.ds(zero(), Dh // 2), :], BF16)
        else:
            av = a_operand(i, hf)
            a_scrs[(i - 1) * NH + hf][...] = pltpu.bitcast(av, U32)
        mi = jnp.dot(av, w.astype(BF16), preferred_element_type=F32)
        if hf > 0:
            mi = mi + st.pop(("part", i))
        results.append((starts[-1], Dh, mi))
        if hf + 1 < NH:
            st[("part", i)] = mi
            return
        col = g * GW + u * 256

        def out(r, cx, x, scale):
            ot_ref[r * Dh:(r + 1) * Dh, col + cx * 128:col + (cx + 1) * 128] = (
                x * rep(scale, Dh)).astype(ot_ref.dtype)

        if i in a_order:
            r_scrs[u * 4 + i - 2][...] = mi
        elif i == 1:
            m2, m3, m4, m5 = (r_scrs[u * 4 + j][pl.ds(zero(), Dh), :] for j in range(4))
            out(1, 0, m2 + m4, st["rx"])
            out(0, 1, m5 - m3, st["ry"])
            st["c11"] = mi + (m4 + rep(st["rho"], Dh) * m5)
            st["c22"] = (m2 - rep(st["rho"], Dh) * m3) - mi
        elif i == 6:
            out(1, 1, st.pop("c22") - mi, st["rx"])
        else:
            out(0, 0, mi + st.pop("c11"), st["rx"])
        if i == B_ORDER[-1]:
            hook("out", col + 256)

    q_jobs = []
    for n, ch in enumerate(chunks):
        if n == 0 and carried:
            q_jobs += [(qk_pass, *ch, 2), (qk_pass, *ch, 1)]
        else:
            q_jobs += [(qk_round, *ch, rnd) for rnd in range(3)]
    pairs = [(g, u) for g in pv_groups for u in range(2)]
    a_jobs = [pr + (i, hf) for pr in pairs for i in a_order for hf in range(NH)]
    b_jobs = [pr + (i, hf) for pr in pairs for i in B_ORDER for hf in range(NH)]
    na, nb = len(a_order) * NH, len(B_ORDER) * NH
    qi = ai = bi = pos = t = 0
    while qi < len(q_jobs) or ai < len(a_jobs) or bi < len(b_jobs):
        tok = prefix[pos] if pos < len(prefix) else cycle[(pos - len(prefix)) % len(cycle)]
        pos += 1
        if tok == "Q" and qi < len(q_jobs):
            fn, *args = q_jobs[qi]
            g, _, _, carry = groups[args[0]]
            assert not (carry and a_jobs) or ai >= 2 * na * (g + 1)
            hook("qk", qi)
            starts.append(t)
            fn(*args)
            qi += 1
            t += CR
        elif tok == "A" and ai < len(a_jobs):
            assert ai // na - bi // nb < 2
            starts.append(t)
            pv(*a_jobs[ai])
            ai += 1
            t += Dh
        elif tok == "B" and bi < len(b_jobs) and ai >= min((bi // nb + 1) * na + 1, len(a_jobs)):
            starts.append(t)
            pv(*b_jobs[bi])
            bi += 1
            t += Dh
        else:
            continue
        hook("job", qi + ai + bi)
    if tail is not None:
        stage_q(tail[0], 0)
        starts.append(t)
        qk_pass(*tail, 3)


def _kernel(q_hbm, k_hbm, v_hbm, o_hbm, in_buf, o_buf, sem_in, sem_pro, sem_out, m_scr, p3_wide,
            *scrs, c):
    H, D, Sq = q_hbm.shape
    Sk = k_hbm.shape[2]
    ng = Sq // GW
    nch = Sk // (2 * CR)
    k_scr, scrs = scrs[:3 * nch], scrs[3 * nch:]
    s_scrs, scrs = scrs[:N_S], scrs[N_S:]
    a_scrs, scrs = scrs[:7 * NH], scrs[7 * NH:]
    q_scrs, scrs = scrs[:6], scrs[6:]
    p3_scrs, scrs = scrs[:N_P3], scrs[N_P3:]
    r_scrs, p_scrs = scrs[:8], scrs[8:]
    pid = pl.program_id(0)
    qa = (AHEAD + 1) * GW

    def start_inputs(h, hn, slot):
        pltpu.make_async_copy(v_hbm.at[h], in_buf.at[slot, 0], sem_in).start()
        pltpu.make_async_copy(q_hbm.at[h, :, qa:], in_buf.at[slot, 1, :, qa:], sem_in).start()
        pltpu.make_async_copy(k_hbm.at[hn], in_buf.at[slot, 2], sem_in).start()
        pltpu.make_async_copy(q_hbm.at[hn, :, :qa], in_buf.at[slot, 1, :, :qa], sem_in).start()

    def wait_inputs(slot):
        pltpu.make_async_copy(in_buf.at[slot], in_buf.at[slot], sem_in).wait()

    common = dict(k_scr=k_scr, s_scrs=s_scrs, a_scrs=a_scrs, q_scrs=q_scrs, p3_scrs=p3_scrs,
                  p3_wide=p3_wide, r_scrs=r_scrs, p_scrs=p_scrs, m_scr=m_scr, c=c, D=D, Sk=Sk)

    @pl.when(pid == 0)
    def _():
        ks = K_FIRST * 2 * CR
        first = [pltpu.make_async_copy(k_hbm.at[0, :, :ks], in_buf.at[1, 2, :, :ks], sem_pro.at[0]),
                 pltpu.make_async_copy(q_hbm.at[0, :, :GW], in_buf.at[1, 1, :, :GW], sem_pro.at[1])]
        second = [pltpu.make_async_copy(k_hbm.at[0, :, ks:], in_buf.at[1, 2, :, ks:], sem_pro.at[2]),
                  pltpu.make_async_copy(q_hbm.at[0, :, GW:qa], in_buf.at[1, 1, :, GW:qa], sem_pro.at[3])]
        for cp in first + second:
            cp.start()
        start_inputs(0, 1, 0)
        for cp in first:
            cp.wait()
        groups0 = [(g, in_buf.at[1, 1], in_buf.at[1, 2] if g == 0 else None, True)
                   for g in range(AHEAD + 1)]
        chunks0 = ([(g, i) for g in range(AHEAD) for i in range(K_FIRST)]
                   + [(g, i) for g in range(AHEAD) for i in range(K_FIRST, nch)])

        def hook0(kind, x):
            if kind == "qk" and x == 3 * K_FIRST:
                for cp in second:
                    cp.wait()

        _emit(chunks0, (AHEAD, 0), [], groups0, plan=("", "Q", (), 0, 0), carried=False, fwd=True,
              seed=pid, vt_ref=None, ot_ref=None, hook=hook0, **common)

        def body(h, carry):
            slot = lax.bitwise_and(h, 1)
            cur = in_buf.at[slot]
            wait_inputs(slot)

            def hook(kind, x):
                if kind == "job" and x == DMA_AT:
                    start_inputs(h + 1, jnp.minimum(h + 2, H - 1), 1 - slot)

            groups = ([(g, cur.at[1], None, False) for g in range(AHEAD, ng)]
                      + [(g, cur.at[1], cur.at[2] if g == 0 else None, True)
                         for g in range(AHEAD + 1)])
            chunks = [(gi, i) for gi in range(ng) for i in range(nch)]
            _emit(chunks, (ng, 0), list(range(ng)), groups, plan=MAIN_PLAN, carried=True,
                  fwd=False, seed=h, vt_ref=cur.at[0], ot_ref=o_buf.at[h], hook=hook,
                  **common)
            pltpu.make_async_copy(o_buf.at[h], o_hbm.at[h], sem_out).start()
            return carry

        lax.fori_loop(0, H - 1, body, 0)

    @pl.when(pid == 1)
    def _():
        slot = (H - 1) % 2
        wait_inputs(slot)
        edges = [0, *LAST_EDGES, Sq]

        def hook(kind, col):
            if kind == "out" and col in edges[1:]:
                a = edges[edges.index(col) - 1]
                pltpu.make_async_copy(o_buf.at[H - 1, :, a:col], o_hbm.at[H - 1, :, a:col],
                                      sem_out).start()

        groups = [(g, in_buf.at[slot, 1], None, False) for g in range(AHEAD, ng)]
        chunks = [(gi, i) for gi in range(ng - AHEAD) for i in range(nch)]
        _emit(chunks, None, list(range(ng)), groups, plan=LAST_PLAN, carried=True, fwd=False,
              seed=pid, vt_ref=in_buf.at[slot, 0], ot_ref=o_buf.at[H - 1], hook=hook,
              **common)
        pltpu.make_async_copy(o_buf, o_hbm, sem_out).wait()


@jax.jit
def pallas_standalone__mha_softmax__prompt_kernel(
    q: jax.Array,
    k: jax.Array,
    v: jax.Array,
):
    B, H, Sq, D = q.shape
    Sk = k.shape[2]
    BH = B * H
    assert D == 192 and Sq == Sk == N_S * GW and BH >= 2
    c = D ** -0.5 * math.log2(math.e)
    R = Sk // 2 // NH
    qt, kt, vt = (jnp.swapaxes(x, 2, 3).reshape(BH, D, Sq) for x in (q, k, v))
    scratch = (
        [pltpu.VMEM((2, 3, D, Sq), BF16),
         pltpu.VMEM((BH, D, Sq), BF16),
         pltpu.SemaphoreType.DMA(()),
         pltpu.SemaphoreType.DMA((4,)),
         pltpu.SemaphoreType.DMA(()),
         pltpu.VMEM((AHEAD * 8, GW), F32),
         pltpu.VMEM((CR, GW + PAD), F32)]
        + [pltpu.VMEM((CR // 2, 2 * D // 3), U32)] * (3 * Sk // (2 * CR))
        + [pltpu.VMEM((Sk, GW + PAD), F32)] * N_S
        + [pltpu.VMEM((D // 4, R), U32)] * (7 * NH)
        + [pltpu.VMEM((D // 6, GW + PAD), U32)] * 6
        + [pltpu.VMEM((CR, 128), F32)] * N_P3
        + [pltpu.VMEM((D // 2, 128), F32)] * 8
        + [pltpu.VMEM((R, 128), F32)] * (8 * NH)
    )
    ot = pl.pallas_call(
        functools.partial(_kernel, c=c),
        grid=(2,),
        in_specs=[pl.BlockSpec(memory_space=pl.ANY)] * 3,
        out_specs=pl.BlockSpec(memory_space=pl.ANY),
        out_shape=jax.ShapeDtypeStruct((BH, D, Sq), q.dtype),
        scratch_shapes=scratch,
        compiler_params=pltpu.CompilerParams(
            dimension_semantics=("arbitrary",),
            vmem_limit_bytes=100 * 1024 * 1024,
            disable_bounds_checks=True,
        ),
    )(qt, kt, vt)
    return jnp.swapaxes(ot.reshape(B, H, D, Sq), 2, 3)
```

```python
import functools
import math

import jax
import jax.numpy as jnp
from jax import lax
import jax.experimental.pallas as pl
import jax.experimental.pallas.tpu as pltpu

F32 = jnp.float32
BF16 = jnp.bfloat16
U32 = jnp.uint32

GW = 512
CR = 128
NH = 2
PAD = 128
S_PAD = 384
AHEAD = 2
N_S = 4
N_P3 = 2
N_SUM = 5
B_ORDER = (1, 7, 6)
MAIN_PLAN = ("QA" + "QQA" * 7, "QQAQBAQQA" + "QBA" * 5, (2, 5, 4, 3), 226, 266)
LAST_PLAN = ("QQA" * 8, "QAA" + "QBA" * 6, (5, 3, 2, 4), 186, 178)
QK_WINDOW = 400
DMA_AT = 4
K_FIRST = 4
LAST_EDGES = (1536, 1792)


def _emit(chunks, tail, pv_groups, groups, *, plan, carried, fwd, seed, vt_ref, ot_ref, hook,
          k_scr, s_scrs, a_scrs, q_scrs, p3_scrs, p3_wide, r_scrs, p_scrs, m_scr, c, D, Sk):
    T = D // 3
    Dh = D // 2
    R = Sk // 2 // NH
    prefix, cycle, a_order, a_tie, b_tie = plan
    cnt = [0]

    def zero():
        cnt[0] += 1
        if carried and cnt[0] <= 3:
            return 0
        return pl.multiple_of(lax.shift_right_logical(seed + cnt[0], 20), 8)

    def rep(x, rows):
        return jnp.concatenate([x] * (rows // 8), axis=0)

    starts = []
    results = []

    def tie(x, dist):
        t = starts[-3] if len(starts) >= 3 else starts[-1]
        recent_qk = any(rows == CR and t - dist - QK_WINDOW <= ts <= t - dist
                        for (ts, rows, _) in results)
        for (ts, rows, val) in reversed(results):
            if ts <= t - dist and (rows == CR or not recent_qk):
                rr = min((t - dist - ts) // 8 * 8, rows - 8)
                a = val[rr:rr + 8, :128]
                return jnp.where(a > jnp.inf, a, x)
        return x

    run_max = {}
    tiles_done = {}
    m_fin = {}
    staged_q = set()
    fwd_k = {}
    q_parts = {1: (0, 1), 2: (0, 2), 3: (1, 2)}
    if carried:
        staged_q.update({(chunks[0][0], j) for j in range(3)})

    def prep_k(gi, i):
        kt_ref = groups[gi][2]
        a = kt_ref[:, 2 * i * CR:(2 * i + 1) * CR]
        b = kt_ref[:, (2 * i + 1) * CR:(2 * i + 2) * CR]
        x = (a[T:2 * T].astype(F32) - b[T:2 * T].astype(F32)).astype(BF16)
        y = (b[2 * T:].astype(F32) - a[2 * T:].astype(F32)).astype(BF16)
        lhs = {1: jnp.concatenate([a[:T], x], axis=0).T,
               2: jnp.concatenate([b[:T], y], axis=0).T,
               3: jnp.concatenate([b[T:2 * T], a[2 * T:]], axis=0).T}
        for w, l in lhs.items():
            k_scr[3 * i + w - 1][...] = pltpu.bitcast(l, U32)
            if fwd:
                fwd_k[(gi, i, w)] = l

    def stage_q(gi, j):
        g, qt_ref = groups[gi][:2]
        staged_q.add((gi, j))
        qt = qt_ref[j * T:(j + 1) * T, g * GW:(g + 1) * GW]
        q_scrs[3 * (g % 2) + j][:, :GW] = pltpu.bitcast(qt, U32)
        return qt

    def q_third(gi, j):
        if (gi, j) not in staged_q:
            return stage_q(gi, j)
        qs = q_scrs[3 * (groups[gi][0] % 2) + j]
        return pltpu.bitcast(qs[pl.ds(zero(), T // 2), :GW], BF16)

    def k_operand(gi, i, w):
        if (gi, i, w) in fwd_k:
            return fwd_k.pop((gi, i, w))
        return pltpu.bitcast(k_scr[3 * i + w - 1][pl.ds(zero(), CR // 2), :], BF16)

    def finish(gi, i, w, ct, s):
        g, _, _, carry = groups[gi]
        s = s * c
        row = (w - 1) * (Sk // 2) + i * CR
        s_scrs[g % N_S][row:row + CR, ct * 128:ct * 128 + s.shape[1]] = s
        for n in range(s.shape[1] // 128):
            mx = run_max.get((gi, ct + n))
            for rr in range(CR // 8):
                x = s[rr * 8:(rr + 1) * 8, n * 128:(n + 1) * 128]
                mx = x if mx is None else jnp.maximum(mx, x)
            run_max[(gi, ct + n)] = mx
        tiles_done[gi] = tiles_done.get(gi, 0) + s.shape[1] // 128
        if tiles_done[gi] == (Sk // CR) * (GW // 128):
            mx = jnp.concatenate([run_max[(gi, n)] for n in range(GW // 128)], axis=1)
            m = jnp.broadcast_to(jnp.max(mx, axis=0, keepdims=True), (8, GW))
            if carry:
                m_scr[g * 8:(g + 1) * 8, :] = m
            else:
                m_fin[g] = m

    def qk_pass(gi, i, w):
        wt = jnp.concatenate([q_third(gi, j) for j in q_parts[w]], axis=0)
        pw = jnp.dot(k_operand(gi, i, w), wt, preferred_element_type=F32)
        results.append((starts[-1], CR, pw))
        if w == 3:
            p3_wide[:, :GW] = pw
        else:
            finish(gi, i, w, 0, pw + p3_wide[pl.ds(zero(), CR), :GW])

    def qk_round(gi, i, rnd):
        qv = [q_third(gi, j) for j in range(3)]
        if groups[gi][2] is not None and rnd == 0:
            prep_k(gi, i)
        kk = {w: k_operand(gi, i, w) for w in (1, 2, 3)}

        def dot(w, ct):
            wt = jnp.concatenate([qv[j][:, ct * 128:(ct + 1) * 128] for j in q_parts[w]], axis=0)
            return jnp.dot(kk[w], wt, preferred_element_type=F32)

        p3 = dot(3, rnd)
        results.append((starts[-1], CR, p3))
        finish(gi, i, 1, rnd, dot(1, rnd) + p3)
        finish(gi, i, 2, rnd, dot(2, rnd) + p3)
        if rnd == 0:
            p3_scrs[i % N_P3][...] = dot(3, 3)
        else:
            finish(gi, i, rnd, 3, dot(rnd, 3) + p3_scrs[i % N_P3][pl.ds(zero(), CR), :])

    s_off = {}
    state = {}

    def a_operand(i, hf):
        tiles = []
        for kp in range(hf * R // 128, (hf + 1) * R // 128):
            def blk(r, kr):
                return vt_ref[r * Dh:(r + 1) * Dh, (2 * kp + kr) * 128:(2 * kp + kr + 1) * 128]

            def add(x, y):
                return (blk(*x).astype(F32) + blk(*y).astype(F32)).astype(BF16)

            def sub(x, y):
                return (blk(*x).astype(F32) - blk(*y).astype(F32)).astype(BF16)

            tiles.append({1: lambda: add((0, 0), (1, 1)), 2: lambda: add((1, 0), (1, 1)),
                          3: lambda: blk(0, 0), 4: lambda: blk(1, 1),
                          5: lambda: add((0, 0), (0, 1)), 6: lambda: sub((1, 0), (0, 0)),
                          7: lambda: sub((0, 1), (1, 1))}[i]())
        return jnp.concatenate(tiles, axis=1)

    def pv(g, u, i, hf):
        if g not in s_off:
            s_off[g] = zero()
            if g < AHEAD:
                m_fin[g] = m_scr[g * 8:(g + 1) * 8, :]
        st = state.setdefault((g, u), {})

        def pbuf(kr, cx):
            return p_scrs[(u * 4 + kr * 2 + cx) * NH + hf]

        def fresh(kr, cx):
            cs = slice((2 * u + cx) * 128, (2 * u + cx + 1) * 128)
            s = s_scrs[g % N_S][pl.ds(s_off[g] + kr * (Sk // 2) + hf * R, R), cs]
            p = jnp.exp2(s - rep(tie(m_fin[g][:, cs], a_tie), R))
            pbuf(kr, cx)[...] = p
            return p

        def load(kr, cx):
            return pbuf(kr, cx)[pl.ds(zero(), R), :]

        def eager_sum(cx, p):
            la = st.get(("l", cx), [None] * 4)
            for tt in range(R // 128):
                for ii in range(7, -1, -1):
                    rr = tt * 128 + ii * 16
                    v = p[rr:rr + 8] + p[rr + 8:rr + 16]
                    la[tt % 4] = v if la[tt % 4] is None else la[tt % 4] + v
            if hf + 1 == NH:
                la = [(la[0] + la[1]) + (la[2] + la[3])] + [None] * (N_SUM - 1)
            st[("l", cx)] = la

        def lazy_sum(kr, cx):
            x = load(kr, cx)
            la = st[("l", cx)]
            for rr in range(R // 8):
                v = x[rr * 8:(rr + 1) * 8]
                la[rr % N_SUM] = v if la[rr % N_SUM] is None else la[rr % N_SUM] + v

        def total(cx):
            l8 = functools.reduce(lambda a, b: a + b, st[("l", cx)])
            return jnp.broadcast_to(jnp.sum(l8, axis=0, keepdims=True), (8, 128))

        def cross(kx, ky):
            if "rho" not in st:
                lx = total(0)
                st["rx"] = 1.0 / lx
                st["ry"] = 1.0 / total(1)
                st["rho"] = lx * st["ry"]
            rho = tie(st["rho"], b_tie)
            return load(kx, 0) - rep(rho, R) * load(ky, 1)

        if i == 2:
            w = fresh(0, 0)
            eager_sum(0, w)
        elif i == 4:
            w = fresh(1, 0) - load(0, 0)
            lazy_sum(1, 0)
        elif i == 5:
            w = fresh(1, 1)
            eager_sum(1, w)
        elif i == 3:
            w = load(1, 1) - fresh(0, 1)
            lazy_sum(0, 1)
        else:
            w = cross(*{1: (0, 1), 6: (0, 0), 7: (1, 1)}[i])
        if (g, u) != (0, 0):
            av = pltpu.bitcast(a_scrs[(i - 1) * NH + hf][pl.ds(zero(), Dh // 2), :], BF16)
        else:
            av = a_operand(i, hf)
            a_scrs[(i - 1) * NH + hf][...] = pltpu.bitcast(av, U32)
        mi = jnp.dot(av, w.astype(BF16), preferred_element_type=F32)
        if hf > 0:
            mi = mi + st.pop(("part", i))
        results.append((starts[-1], Dh, mi))
        if hf + 1 < NH:
            st[("part", i)] = mi
            return
        col = g * GW + u * 256

        def out(r, cx, x, scale):
            ot_ref[r * Dh:(r + 1) * Dh, col + cx * 128:col + (cx + 1) * 128] = (
                x * rep(scale, Dh)).astype(ot_ref.dtype)
            hook("tile", (r * Dh, col + cx * 128))

        if i in a_order:
            r_scrs[u * 4 + i - 2][...] = mi
        elif i == 1:
            m2, m3, m4, m5 = (r_scrs[u * 4 + j][pl.ds(zero(), Dh), :] for j in range(4))
            out(1, 0, m2 + m4, st["rx"])
            out(0, 1, m5 - m3, st["ry"])
            st["c11"] = mi + (m4 + rep(st["rho"], Dh) * m5)
            st["c22"] = (m2 - rep(st["rho"], Dh) * m3) - mi
        elif i == 6:
            out(1, 1, st.pop("c22") - mi, st["rx"])
        else:
            out(0, 0, mi + st.pop("c11"), st["rx"])
        if i == B_ORDER[-1]:
            hook("out", col + 256)

    q_jobs = []
    for n, ch in enumerate(chunks):
        if n == 0 and carried:
            q_jobs += [(qk_pass, *ch, 2), (qk_pass, *ch, 1)]
        else:
            q_jobs += [(qk_round, *ch, rnd) for rnd in range(3)]
    pairs = [(g, u) for g in pv_groups for u in range(2)]
    a_jobs = [pr + (i, hf) for pr in pairs for i in a_order for hf in range(NH)]
    b_jobs = [pr + (i, hf) for pr in pairs for i in B_ORDER for hf in range(NH)]
    na, nb = len(a_order) * NH, len(B_ORDER) * NH
    qi = ai = bi = pos = t = 0
    while qi < len(q_jobs) or ai < len(a_jobs) or bi < len(b_jobs):
        tok = prefix[pos] if pos < len(prefix) else cycle[(pos - len(prefix)) % len(cycle)]
        pos += 1
        if tok == "Q" and qi < len(q_jobs):
            fn, *args = q_jobs[qi]
            g, _, _, carry = groups[args[0]]
            assert not (carry and a_jobs) or ai >= 2 * na * (g + 1)
            hook("qk", qi)
            starts.append(t)
            fn(*args)
            qi += 1
            t += CR
        elif tok == "A" and ai < len(a_jobs):
            assert ai // na - bi // nb < 2
            starts.append(t)
            pv(*a_jobs[ai])
            ai += 1
            t += Dh
        elif tok == "B" and bi < len(b_jobs) and ai >= min((bi // nb + 1) * na + 1, len(a_jobs)):
            starts.append(t)
            pv(*b_jobs[bi])
            bi += 1
            t += Dh
        else:
            continue
        hook("job", qi + ai + bi)
    if tail is not None:
        stage_q(tail[0], 0)
        starts.append(t)
        qk_pass(*tail, 3)


def _kernel(q_hbm, k_hbm, v_hbm, o_hbm, in_buf, o_buf, sem_in, sem_pro, sem_out, m_scr, p3_wide,
            *scrs, c):
    H, D, Sq = q_hbm.shape
    Sk = k_hbm.shape[2]
    ng = Sq // GW
    nch = Sk // (2 * CR)
    k_scr, scrs = scrs[:3 * nch], scrs[3 * nch:]
    s_scrs, scrs = scrs[:N_S], scrs[N_S:]
    a_scrs, scrs = scrs[:7 * NH], scrs[7 * NH:]
    q_scrs, scrs = scrs[:6], scrs[6:]
    p3_scrs, scrs = scrs[:N_P3], scrs[N_P3:]
    r_scrs, p_scrs = scrs[:8], scrs[8:]
    pid = pl.program_id(0)
    qa = (AHEAD + 1) * GW

    def start_inputs(h, hn, slot):
        pltpu.make_async_copy(v_hbm.at[h], in_buf.at[slot, 0], sem_in).start()
        pltpu.make_async_copy(q_hbm.at[h, :, qa:], in_buf.at[slot, 1, :, qa:], sem_in).start()
        pltpu.make_async_copy(k_hbm.at[hn], in_buf.at[slot, 2], sem_in).start()
        pltpu.make_async_copy(q_hbm.at[hn, :, :qa], in_buf.at[slot, 1, :, :qa], sem_in).start()

    def wait_inputs(slot):
        pltpu.make_async_copy(in_buf.at[slot], in_buf.at[slot], sem_in).wait()

    common = dict(k_scr=k_scr, s_scrs=s_scrs, a_scrs=a_scrs, q_scrs=q_scrs, p3_scrs=p3_scrs,
                  p3_wide=p3_wide, r_scrs=r_scrs, p_scrs=p_scrs, m_scr=m_scr, c=c, D=D, Sk=Sk)

    @pl.when(pid == 0)
    def _():
        ks = K_FIRST * 2 * CR
        first = [pltpu.make_async_copy(k_hbm.at[0, :, :ks], in_buf.at[1, 2, :, :ks], sem_pro.at[0]),
                 pltpu.make_async_copy(q_hbm.at[0, :, :GW], in_buf.at[1, 1, :, :GW], sem_pro.at[1])]
        second = [pltpu.make_async_copy(k_hbm.at[0, :, ks:], in_buf.at[1, 2, :, ks:], sem_pro.at[2]),
                  pltpu.make_async_copy(q_hbm.at[0, :, GW:qa], in_buf.at[1, 1, :, GW:qa], sem_pro.at[3])]
        for cp in first + second:
            cp.start()
        start_inputs(0, 1, 0)
        for cp in first:
            cp.wait()
        groups0 = [(g, in_buf.at[1, 1], in_buf.at[1, 2] if g == 0 else None, True)
                   for g in range(AHEAD + 1)]
        chunks0 = ([(g, i) for g in range(AHEAD) for i in range(K_FIRST)]
                   + [(g, i) for g in range(AHEAD) for i in range(K_FIRST, nch)])

        def hook0(kind, x):
            if kind == "qk" and x == 3 * K_FIRST:
                for cp in second:
                    cp.wait()

        _emit(chunks0, (AHEAD, 0), [], groups0, plan=("", "Q", (), 0, 0), carried=False, fwd=True,
              seed=pid, vt_ref=None, ot_ref=None, hook=hook0, **common)

        def body(h, carry):
            slot = lax.bitwise_and(h, 1)
            cur = in_buf.at[slot]
            wait_inputs(slot)

            def hook(kind, x):
                if kind == "job" and x == DMA_AT:
                    start_inputs(h + 1, jnp.minimum(h + 2, H - 1), 1 - slot)

            groups = ([(g, cur.at[1], None, False) for g in range(AHEAD, ng)]
                      + [(g, cur.at[1], cur.at[2] if g == 0 else None, True)
                         for g in range(AHEAD + 1)])
            chunks = [(gi, i) for gi in range(ng) for i in range(nch)]
            _emit(chunks, (ng, 0), list(range(ng)), groups, plan=MAIN_PLAN, carried=True,
                  fwd=False, seed=h, vt_ref=cur.at[0], ot_ref=o_buf.at[h], hook=hook,
                  **common)
            pltpu.make_async_copy(o_buf.at[h], o_hbm.at[h], sem_out).start()
            return carry

        lax.fori_loop(0, H - 1, body, 0)

    @pl.when(pid == 1)
    def _():
        slot = (H - 1) % 2
        wait_inputs(slot)
        edges = [0, *LAST_EDGES]

        def hook(kind, x):
            if kind == "out" and x in edges[1:]:
                idx = (H - 1, slice(None), slice(edges[edges.index(x) - 1], x))
            elif kind == "tile" and x[1] >= edges[-1]:
                idx = (H - 1, slice(x[0], x[0] + D // 2), slice(x[1], x[1] + 128))
            else:
                return
            pltpu.make_async_copy(o_buf.at[idx], o_hbm.at[idx], sem_out).start()

        groups = [(g, in_buf.at[slot, 1], None, False) for g in range(AHEAD, ng)]
        chunks = [(gi, i) for gi in range(ng - AHEAD) for i in range(nch)]
        _emit(chunks, None, list(range(ng)), groups, plan=LAST_PLAN, carried=True, fwd=False,
              seed=pid, vt_ref=in_buf.at[slot, 0], ot_ref=o_buf.at[H - 1], hook=hook,
              **common)
        pltpu.make_async_copy(o_buf, o_hbm, sem_out).wait()


@jax.jit
def pallas_standalone__mha_softmax__prompt_kernel(
    q: jax.Array,
    k: jax.Array,
    v: jax.Array,
):
    B, H, Sq, D = q.shape
    Sk = k.shape[2]
    BH = B * H
    assert D == 192 and Sq == Sk == N_S * GW and BH >= 2
    c = D ** -0.5 * math.log2(math.e)
    R = Sk // 2 // NH
    qt, kt, vt = (jnp.swapaxes(x, 2, 3).reshape(BH, D, Sq) for x in (q, k, v))
    scratch = (
        [pltpu.VMEM((2, 3, D, Sq), BF16),
         pltpu.VMEM((BH, D, Sq), BF16),
         pltpu.SemaphoreType.DMA(()),
         pltpu.SemaphoreType.DMA((4,)),
         pltpu.SemaphoreType.DMA(()),
         pltpu.VMEM((AHEAD * 8, GW), F32),
         pltpu.VMEM((CR, GW + PAD), F32)]
        + [pltpu.VMEM((CR // 2, 2 * D // 3), U32)] * (3 * Sk // (2 * CR))
        + [pltpu.VMEM((Sk, GW + S_PAD), F32)] * N_S
        + [pltpu.VMEM((D // 4, R), U32)] * (7 * NH)
        + [pltpu.VMEM((D // 6, GW + PAD), U32)] * 6
        + [pltpu.VMEM((CR, 128), F32)] * N_P3
        + [pltpu.VMEM((D // 2, 128), F32)] * 8
        + [pltpu.VMEM((R, 128), F32)] * (8 * NH)
    )
    ot = pl.pallas_call(
        functools.partial(_kernel, c=c),
        grid=(2,),
        in_specs=[pl.BlockSpec(memory_space=pl.ANY)] * 3,
        out_specs=pl.BlockSpec(memory_space=pl.ANY),
        out_shape=jax.ShapeDtypeStruct((BH, D, Sq), q.dtype),
        scratch_shapes=scratch,
        compiler_params=pltpu.CompilerParams(
            dimension_semantics=("arbitrary",),
            vmem_limit_bytes=100 * 1024 * 1024,
            disable_bounds_checks=True,
        ),
    )(qt, kt, vt)
    return jnp.swapaxes(ot.reshape(B, H, D, Sq), 2, 3)
```

```python
import functools
import math

import jax
import jax.numpy as jnp
from jax import lax
import jax.experimental.pallas as pl
import jax.experimental.pallas.tpu as pltpu

F32 = jnp.float32
BF16 = jnp.bfloat16
U32 = jnp.uint32

GW = 512
CR = 128
NH = 2
PAD = 128
AHEAD = 2
N_S = 4
N_P3 = 4
N_SUM = 4
B_ORDER = (1, 6, 7)
MAIN_PLAN = ("QA" * 2 + "QQA" * 6, "QQA" * 2 + "QBA" * 6, (2, 5, 4, 3), 210, 194)
LAST_PLAN = ("QQA" * 8, "QAA" + "QBA" * 6, (5, 3, 2, 4), 186, 178)
QK_WINDOW = 400
STAGGER = (32, 48, 64, 80)
DMA_AT = 40
K_FIRST = 4
LAST_EDGES = (1536, 1792)


def _emit(chunks, tail, pv_groups, groups, *, plan, carried, fwd, seed, vt_ref, ot_ref, hook,
          k_scr, s_scrs, a_scrs, q_scrs, p3_scrs, p3_wide, r_scrs, p_scrs, m_scr, c, D, Sk):
    T = D // 3
    Dh = D // 2
    R = Sk // 2 // NH
    prefix, cycle, a_order, a_tie, b_tie = plan
    cnt = [0]

    def zero():
        cnt[0] += 1
        if carried and cnt[0] <= 3:
            return 0
        return pl.multiple_of(lax.shift_right_logical(seed + cnt[0], 20), 8)

    def rep(x, rows):
        return jnp.concatenate([x] * (rows // 8), axis=0)

    starts = []
    results = []

    def tie(x, dist):
        t = starts[-3] if len(starts) >= 3 else starts[-1]
        recent_qk = any(rows == CR and t - dist - QK_WINDOW <= ts <= t - dist
                        for (ts, rows, _) in results)
        for (ts, rows, val) in reversed(results):
            if ts <= t - dist and (rows == CR or not recent_qk):
                rr = min((t - dist - ts) // 8 * 8, rows - 8)
                a = val[rr:rr + 8, :128]
                return jnp.where(a > jnp.inf, a, x)
        return x

    run_max = {}
    tiles_done = {}
    m_fin = {}
    staged_q = set()
    fwd_k = {}
    q_parts = {1: (0, 1), 2: (0, 2), 3: (1, 2)}
    if carried:
        staged_q.update({(chunks[0][0], j) for j in range(3)})

    def prep_k(gi, i):
        kt_ref = groups[gi][2]
        a = kt_ref[:, 2 * i * CR:(2 * i + 1) * CR]
        b = kt_ref[:, (2 * i + 1) * CR:(2 * i + 2) * CR]
        x = (a[T:2 * T].astype(F32) - b[T:2 * T].astype(F32)).astype(BF16)
        y = (b[2 * T:].astype(F32) - a[2 * T:].astype(F32)).astype(BF16)
        lhs = {1: jnp.concatenate([a[:T], x], axis=0).T,
               2: jnp.concatenate([b[:T], y], axis=0).T,
               3: jnp.concatenate([b[T:2 * T], a[2 * T:]], axis=0).T}
        for w, l in lhs.items():
            k_scr[3 * i + w - 1][...] = pltpu.bitcast(l, U32)
            if fwd:
                fwd_k[(gi, i, w)] = l

    def stage_q(gi, j):
        g, qt_ref = groups[gi][:2]
        staged_q.add((gi, j))
        qt = qt_ref[j * T:(j + 1) * T, g * GW:(g + 1) * GW]
        q_scrs[3 * (g % 2) + j][:, :GW] = pltpu.bitcast(qt, U32)
        return qt

    def q_third(gi, j):
        if (gi, j) not in staged_q:
            return stage_q(gi, j)
        qs = q_scrs[3 * (groups[gi][0] % 2) + j]
        return pltpu.bitcast(qs[pl.ds(zero(), T // 2), :GW], BF16)

    def k_operand(gi, i, w):
        if (gi, i, w) in fwd_k:
            return fwd_k.pop((gi, i, w))
        return pltpu.bitcast(k_scr[3 * i + w - 1][pl.ds(zero(), CR // 2), :], BF16)

    def finish(gi, i, w, ct, s):
        g, _, _, carry = groups[gi]
        s = s * c
        row = (w - 1) * (Sk // 2) + i * CR
        s_scrs[g % N_S][row:row + CR, ct * 128:ct * 128 + s.shape[1]] = s
        for n in range(s.shape[1] // 128):
            mx = run_max.get((gi, ct + n))
            for rr in range(CR // 8):
                x = s[rr * 8:(rr + 1) * 8, n * 128:(n + 1) * 128]
                mx = x if mx is None else jnp.maximum(mx, x)
            run_max[(gi, ct + n)] = mx
        tiles_done[gi] = tiles_done.get(gi, 0) + s.shape[1] // 128
        if tiles_done[gi] == (Sk // CR) * (GW // 128):
            mx = jnp.concatenate([run_max[(gi, n)] for n in range(GW // 128)], axis=1)
            m = jnp.broadcast_to(jnp.max(mx, axis=0, keepdims=True), (8, GW))
            if carry:
                m_scr[g * 8:(g + 1) * 8, :] = m
            else:
                m_fin[g] = m

    def qk_split(gi, i, head):
        qv = [q_third(gi, j) for j in q_parts[3]]
        kk = k_operand(gi, i, 3)
        for ct in range(GW // 128):
            lo, hi = (CR - STAGGER[ct], CR) if head else (0, CR - STAGGER[ct])
            wt = jnp.concatenate([x[:, ct * 128:(ct + 1) * 128] for x in qv], axis=0)
            p3_wide[lo:hi, ct * 128:(ct + 1) * 128] = jnp.dot(kk[lo:hi], wt,
                                                              preferred_element_type=F32)

    def qk_pass(gi, i, w):
        wt = jnp.concatenate([q_third(gi, j) for j in q_parts[w]], axis=0)
        pw = jnp.dot(k_operand(gi, i, w), wt, preferred_element_type=F32)
        results.append((starts[-1], CR, pw))
        finish(gi, i, w, 0, pw + p3_wide[pl.ds(zero(), CR), :GW])

    def qk_round(gi, i, rnd):
        qv = [q_third(gi, j) for j in range(3)]
        if groups[gi][2] is not None and rnd == 0:
            prep_k(gi, i)
        kk = {w: k_operand(gi, i, w) for w in (1, 2, 3)}

        def dot(w, ct):
            wt = jnp.concatenate([qv[j][:, ct * 128:(ct + 1) * 128] for j in q_parts[w]], axis=0)
            return jnp.dot(kk[w], wt, preferred_element_type=F32)

        p3 = dot(3, rnd)
        results.append((starts[-1], CR, p3))
        finish(gi, i, 1, rnd, dot(1, rnd) + p3)
        finish(gi, i, 2, rnd, dot(2, rnd) + p3)
        if rnd == 0:
            p3_scrs[i % N_P3][...] = dot(3, 3)
        else:
            finish(gi, i, rnd, 3, dot(rnd, 3) + p3_scrs[i % N_P3][pl.ds(zero(), CR), :])

    s_off = {}
    state = {}

    def a_operand(i, hf):
        tiles = []
        for kp in range(hf * R // 128, (hf + 1) * R // 128):
            def blk(r, kr):
                return vt_ref[r * Dh:(r + 1) * Dh, (2 * kp + kr) * 128:(2 * kp + kr + 1) * 128]

            def add(x, y):
                return (blk(*x).astype(F32) + blk(*y).astype(F32)).astype(BF16)

            def sub(x, y):
                return (blk(*x).astype(F32) - blk(*y).astype(F32)).astype(BF16)

            tiles.append({1: lambda: add((0, 0), (1, 1)), 2: lambda: add((1, 0), (1, 1)),
                          3: lambda: blk(0, 0), 4: lambda: blk(1, 1),
                          5: lambda: add((0, 0), (0, 1)), 6: lambda: sub((1, 0), (0, 0)),
                          7: lambda: sub((0, 1), (1, 1))}[i]())
        return jnp.concatenate(tiles, axis=1)

    def pv(g, u, i, hf):
        if g not in s_off:
            s_off[g] = zero()
            if g < AHEAD:
                m_fin[g] = m_scr[g * 8:(g + 1) * 8, :]
        st = state.setdefault((g, u), {})

        def pbuf(kr, cx):
            return p_scrs[(u * 4 + kr * 2 + cx) * NH + hf]

        def fresh(kr, cx):
            cs = slice((2 * u + cx) * 128, (2 * u + cx + 1) * 128)
            s = s_scrs[g % N_S][pl.ds(s_off[g] + kr * (Sk // 2) + hf * R, R), cs]
            p = jnp.exp2(s - rep(tie(m_fin[g][:, cs], a_tie), R))
            pbuf(kr, cx)[...] = p
            return p

        def load(kr, cx):
            return pbuf(kr, cx)[pl.ds(zero(), R), :]

        def eager_sum(cx, p):
            la = st.get(("l", cx), [None] * 4)
            for tt in range(R // 128):
                for ii in range(7, -1, -1):
                    rr = tt * 128 + ii * 16
                    v = p[rr:rr + 8] + p[rr + 8:rr + 16]
                    la[tt % 4] = v if la[tt % 4] is None else la[tt % 4] + v
            if hf + 1 == NH:
                la = [(la[0] + la[1]) + (la[2] + la[3])] + [None] * (N_SUM - 1)
            st[("l", cx)] = la

        def lazy_sum(kr, cx):
            x = load(kr, cx)
            la = st[("l", cx)]
            for rr in range(R // 8):
                v = x[rr * 8:(rr + 1) * 8]
                la[rr % N_SUM] = v if la[rr % N_SUM] is None else la[rr % N_SUM] + v

        def total(cx):
            l8 = functools.reduce(lambda a, b: a + b, st[("l", cx)])
            return jnp.broadcast_to(jnp.sum(l8, axis=0, keepdims=True), (8, 128))

        def cross(kx, ky):
            if "rho" not in st:
                lx = total(0)
                st["rx"] = 1.0 / lx
                st["ry"] = 1.0 / total(1)
                st["rho"] = lx * st["ry"]
            rho = tie(st["rho"], b_tie)
            return load(kx, 0) - rep(rho, R) * load(ky, 1)

        if i == 2:
            w = fresh(0, 0)
            eager_sum(0, w)
        elif i == 4:
            w = fresh(1, 0) - load(0, 0)
            lazy_sum(1, 0)
        elif i == 5:
            w = fresh(1, 1)
            eager_sum(1, w)
        elif i == 3:
            w = load(1, 1) - fresh(0, 1)
            lazy_sum(0, 1)
        else:
            w = cross(*{1: (0, 1), 6: (0, 0), 7: (1, 1)}[i])
        if (g, u) != (0, 0):
            av = pltpu.bitcast(a_scrs[(i - 1) * NH + hf][pl.ds(zero(), Dh // 2), :], BF16)
        else:
            av = a_operand(i, hf)
            a_scrs[(i - 1) * NH + hf][...] = pltpu.bitcast(av, U32)
        mi = jnp.dot(av, w.astype(BF16), preferred_element_type=F32)
        if hf > 0:
            mi = mi + st.pop(("part", i))
        results.append((starts[-1], Dh, mi))
        if hf + 1 < NH:
            st[("part", i)] = mi
            return
        col = g * GW + u * 256

        def out(r, cx, x, scale):
            ot_ref[r * Dh:(r + 1) * Dh, col + cx * 128:col + (cx + 1) * 128] = (
                x * rep(scale, Dh)).astype(ot_ref.dtype)
            hook("tile", (r * Dh, col + cx * 128))

        if i in a_order:
            r_scrs[u * 4 + i - 2][...] = mi
        elif i == 1:
            m2, m3, m4, m5 = (r_scrs[u * 4 + j][pl.ds(zero(), Dh), :] for j in range(4))
            out(1, 0, m2 + m4, st["rx"])
            out(0, 1, m5 - m3, st["ry"])
            st["c11"] = mi + (m4 + rep(st["rho"], Dh) * m5)
            st["c22"] = (m2 - rep(st["rho"], Dh) * m3) - mi
        elif i == 6:
            out(1, 1, st.pop("c22") - mi, st["rx"])
        else:
            out(0, 0, mi + st.pop("c11"), st["rx"])
        if i == B_ORDER[-1]:
            hook("out", col + 256)

    q_jobs = [(qk_round, *ch, rnd) for ch in chunks[1 if carried else 0:] for rnd in range(3)]
    if carried:
        qk_split(*chunks[0], True)
        q_jobs[3:3] = [(qk_pass, *chunks[0], 2), (qk_pass, *chunks[0], 1)]
    pairs = [(g, u) for g in pv_groups for u in range(2)]
    a_jobs = [pr + (i, hf) for pr in pairs for i in a_order for hf in range(NH)]
    b_jobs = [pr + (i, hf) for pr in pairs for i in B_ORDER for hf in range(NH)]
    na, nb = len(a_order) * NH, len(B_ORDER) * NH
    qi = ai = bi = pos = t = 0
    while qi < len(q_jobs) or ai < len(a_jobs) or bi < len(b_jobs):
        tok = prefix[pos] if pos < len(prefix) else cycle[(pos - len(prefix)) % len(cycle)]
        pos += 1
        if tok == "Q" and qi < len(q_jobs):
            fn, *args = q_jobs[qi]
            g, _, _, carry = groups[args[0]]
            assert not (carry and a_jobs) or ai >= 2 * na * (g + 1)
            hook("qk", qi)
            starts.append(t)
            fn(*args)
            qi += 1
            t += CR
        elif tok == "A" and ai < len(a_jobs):
            assert ai // na - bi // nb < 2
            starts.append(t)
            pv(*a_jobs[ai])
            ai += 1
            t += Dh
        elif tok == "B" and bi < len(b_jobs) and ai >= min((bi // nb + 1) * na + 1, len(a_jobs)):
            starts.append(t)
            pv(*b_jobs[bi])
            bi += 1
            t += Dh
        else:
            continue
        hook("job", qi + ai + bi)
    if tail is not None:
        stage_q(tail[0], 0)
        qk_split(*tail, False)


def _kernel(q_hbm, k_hbm, v_hbm, o_hbm, in_buf, o_buf, sem_in, sem_pro, sem_out, m_scr, p3_wide,
            *scrs, c):
    H, D, Sq = q_hbm.shape
    Sk = k_hbm.shape[2]
    ng = Sq // GW
    nch = Sk // (2 * CR)
    k_scr, scrs = scrs[:3 * nch], scrs[3 * nch:]
    s_scrs, scrs = scrs[:N_S], scrs[N_S:]
    a_scrs, scrs = scrs[:7 * NH], scrs[7 * NH:]
    q_scrs, scrs = scrs[:6], scrs[6:]
    p3_scrs, scrs = scrs[:N_P3], scrs[N_P3:]
    r_scrs, p_scrs = scrs[:8], scrs[8:]
    pid = pl.program_id(0)
    qa = (AHEAD + 1) * GW

    def start_inputs(h, hn, slot):
        pltpu.make_async_copy(v_hbm.at[h], in_buf.at[slot, 0], sem_in).start()
        pltpu.make_async_copy(q_hbm.at[h, :, qa:], in_buf.at[slot, 1, :, qa:], sem_in).start()
        pltpu.make_async_copy(k_hbm.at[hn], in_buf.at[slot, 2], sem_in).start()
        pltpu.make_async_copy(q_hbm.at[hn, :, :qa], in_buf.at[slot, 1, :, :qa], sem_in).start()

    def wait_inputs(slot):
        pltpu.make_async_copy(in_buf.at[slot], in_buf.at[slot], sem_in).wait()

    common = dict(k_scr=k_scr, s_scrs=s_scrs, a_scrs=a_scrs, q_scrs=q_scrs, p3_scrs=p3_scrs,
                  p3_wide=p3_wide, r_scrs=r_scrs, p_scrs=p_scrs, m_scr=m_scr, c=c, D=D, Sk=Sk)

    @pl.when(pid == 0)
    def _():
        ks = K_FIRST * 2 * CR
        first = [pltpu.make_async_copy(k_hbm.at[0, :, :ks], in_buf.at[1, 2, :, :ks], sem_pro.at[0]),
                 pltpu.make_async_copy(q_hbm.at[0, :, :GW], in_buf.at[1, 1, :, :GW], sem_pro.at[1])]
        second = [pltpu.make_async_copy(k_hbm.at[0, :, ks:], in_buf.at[1, 2, :, ks:], sem_pro.at[2]),
                  pltpu.make_async_copy(q_hbm.at[0, :, GW:qa], in_buf.at[1, 1, :, GW:qa], sem_pro.at[3])]
        for cp in first + second:
            cp.start()
        start_inputs(0, 1, 0)
        for cp in first:
            cp.wait()
        groups0 = [(g, in_buf.at[1, 1], in_buf.at[1, 2] if g == 0 else None, True)
                   for g in range(AHEAD + 1)]
        chunks0 = ([(g, i) for g in range(AHEAD) for i in range(K_FIRST)]
                   + [(g, i) for g in range(AHEAD) for i in range(K_FIRST, nch)])

        def hook0(kind, x):
            if kind == "qk" and x == 3 * K_FIRST:
                for cp in second:
                    cp.wait()

        _emit(chunks0, (AHEAD, 0), [], groups0, plan=("", "Q", (), 0, 0), carried=False, fwd=True,
              seed=pid, vt_ref=None, ot_ref=None, hook=hook0, **common)

        def body(h, carry):
            slot = lax.bitwise_and(h, 1)
            cur = in_buf.at[slot]
            wait_inputs(slot)

            def hook(kind, x):
                if kind == "job" and x == DMA_AT:
                    start_inputs(h + 1, jnp.minimum(h + 2, H - 1), 1 - slot)

            groups = ([(g, cur.at[1], None, False) for g in range(AHEAD, ng)]
                      + [(g, cur.at[1], cur.at[2] if g == 0 else None, True)
                         for g in range(AHEAD + 1)])
            chunks = [(gi, i) for gi in range(ng) for i in range(nch)]
            _emit(chunks, (ng, 0), list(range(ng)), groups, plan=MAIN_PLAN, carried=True,
                  fwd=False, seed=h, vt_ref=cur.at[0], ot_ref=o_buf.at[h], hook=hook,
                  **common)
            pltpu.make_async_copy(o_buf.at[h], o_hbm.at[h], sem_out).start()
            return carry

        lax.fori_loop(0, H - 1, body, 0)

    @pl.when(pid == 1)
    def _():
        slot = (H - 1) % 2
        wait_inputs(slot)
        edges = [0, *LAST_EDGES]

        def hook(kind, x):
            if kind == "out" and x in edges[1:]:
                idx = (H - 1, slice(None), slice(edges[edges.index(x) - 1], x))
            elif kind == "tile" and x[1] >= edges[-1]:
                idx = (H - 1, slice(x[0], x[0] + D // 2), slice(x[1], x[1] + 128))
            else:
                return
            pltpu.make_async_copy(o_buf.at[idx], o_hbm.at[idx], sem_out).start()

        groups = [(g, in_buf.at[slot, 1], None, False) for g in range(AHEAD, ng)]
        chunks = [(gi, i) for gi in range(ng - AHEAD) for i in range(nch)]
        _emit(chunks, None, list(range(ng)), groups, plan=LAST_PLAN, carried=True, fwd=False,
              seed=pid, vt_ref=in_buf.at[slot, 0], ot_ref=o_buf.at[H - 1], hook=hook,
              **common)
        pltpu.make_async_copy(o_buf, o_hbm, sem_out).wait()


@jax.jit
def pallas_standalone__mha_softmax__prompt_kernel(
    q: jax.Array,
    k: jax.Array,
    v: jax.Array,
):
    B, H, Sq, D = q.shape
    Sk = k.shape[2]
    BH = B * H
    assert D == 192 and Sq == Sk == N_S * GW and BH >= 2
    c = D ** -0.5 * math.log2(math.e)
    R = Sk // 2 // NH
    qt, kt, vt = (jnp.swapaxes(x, 2, 3).reshape(BH, D, Sq) for x in (q, k, v))
    scratch = (
        [pltpu.VMEM((2, 3, D, Sq), BF16),
         pltpu.VMEM((BH, D, Sq), BF16),
         pltpu.SemaphoreType.DMA(()),
         pltpu.SemaphoreType.DMA((4,)),
         pltpu.SemaphoreType.DMA(()),
         pltpu.VMEM((AHEAD * 8, GW), F32),
         pltpu.VMEM((CR, GW + PAD), F32)]
        + [pltpu.VMEM((CR // 2, 2 * D // 3), U32)] * (3 * Sk // (2 * CR))
        + [pltpu.VMEM((Sk, GW + PAD), F32)] * N_S
        + [pltpu.VMEM((D // 4, R), U32)] * (7 * NH)
        + [pltpu.VMEM((D // 6, GW + PAD), U32)] * 6
        + [pltpu.VMEM((CR, 128), F32)] * N_P3
        + [pltpu.VMEM((D // 2, 128), F32)] * 8
        + [pltpu.VMEM((R, 128), F32)] * (8 * NH)
    )
    ot = pl.pallas_call(
        functools.partial(_kernel, c=c),
        grid=(2,),
        in_specs=[pl.BlockSpec(memory_space=pl.ANY)] * 3,
        out_specs=pl.BlockSpec(memory_space=pl.ANY),
        out_shape=jax.ShapeDtypeStruct((BH, D, Sq), q.dtype),
        scratch_shapes=scratch,
        compiler_params=pltpu.CompilerParams(
            dimension_semantics=("arbitrary",),
            vmem_limit_bytes=100 * 1024 * 1024,
            disable_bounds_checks=True,
        ),
    )(qt, kt, vt)
    return jnp.swapaxes(ot.reshape(B, H, D, Sq), 2, 3)
```

```python
import functools
import math

import jax
import jax.numpy as jnp
from jax import lax
import jax.experimental.pallas as pl
import jax.experimental.pallas.tpu as pltpu

F32 = jnp.float32
BF16 = jnp.bfloat16
U32 = jnp.uint32

GW = 512
CR = 128
NH = 2
PAD = 128
AHEAD = 2
N_S = 4
N_P3 = 4
N_SUM = 4
B_ORDER = (1, 6, 7)
MAIN_PLAN = ("QA" * 2 + "QQA" * 6, "QQA" * 2 + "QBA" * 6, (2, 5, 4, 3), 210, 194)
LAST_PLAN = ("QQA" * 8, "QAA" + "QBA" * 6, (5, 3, 2, 4), 186, 178)
QK_WINDOW = 400
STAGGER = (32, 48, 64, 80)
DMA_AT = 40
K_EARLY = 1
K_FIRST = 4
LAST_EDGES = (1536, 1792)


def _emit(chunks, tail, pv_groups, groups, *, plan, carried, fwd, seed, vt_ref, ot_ref, hook,
          k_scr, s_scrs, a_scrs, q_scrs, p3_scrs, p3_wide, r_scrs, p_scrs, m_scr, c, D, Sk):
    T = D // 3
    Dh = D // 2
    R = Sk // 2 // NH
    prefix, cycle, a_order, a_tie, b_tie = plan
    cnt = [0]

    def zero():
        cnt[0] += 1
        if carried and cnt[0] <= 3:
            return 0
        return pl.multiple_of(lax.shift_right_logical(seed + cnt[0], 20), 8)

    def rep(x, rows):
        return jnp.concatenate([x] * (rows // 8), axis=0)

    starts = []
    results = []

    def tie(x, dist):
        t = starts[-3] if len(starts) >= 3 else starts[-1]
        recent_qk = any(rows == CR and t - dist - QK_WINDOW <= ts <= t - dist
                        for (ts, rows, _) in results)
        for (ts, rows, val) in reversed(results):
            if ts <= t - dist and (rows == CR or not recent_qk):
                rr = min((t - dist - ts) // 8 * 8, rows - 8)
                a = val[rr:rr + 8, :128]
                return jnp.where(a > jnp.inf, a, x)
        return x

    run_max = {}
    tiles_done = {}
    m_fin = {}
    staged_q = set()
    fwd_k = {}
    q_parts = {1: (0, 1), 2: (0, 2), 3: (1, 2)}
    if carried:
        staged_q.update({(chunks[0][0], j) for j in range(3)})

    def prep_k(gi, i):
        kt_ref = groups[gi][2]
        a = kt_ref[:, 2 * i * CR:(2 * i + 1) * CR]
        b = kt_ref[:, (2 * i + 1) * CR:(2 * i + 2) * CR]
        x = (a[T:2 * T].astype(F32) - b[T:2 * T].astype(F32)).astype(BF16)
        y = (b[2 * T:].astype(F32) - a[2 * T:].astype(F32)).astype(BF16)
        lhs = {1: jnp.concatenate([a[:T], x], axis=0).T,
               2: jnp.concatenate([b[:T], y], axis=0).T,
               3: jnp.concatenate([b[T:2 * T], a[2 * T:]], axis=0).T}
        for w, l in lhs.items():
            k_scr[3 * i + w - 1][...] = pltpu.bitcast(l, U32)
            if fwd:
                fwd_k[(gi, i, w)] = l

    def stage_q(gi, j):
        g, qt_ref = groups[gi][:2]
        staged_q.add((gi, j))
        qt = qt_ref[j * T:(j + 1) * T, g * GW:(g + 1) * GW]
        q_scrs[3 * (g % 2) + j][:, :GW] = pltpu.bitcast(qt, U32)
        return qt

    def q_third(gi, j):
        if (gi, j) not in staged_q:
            return stage_q(gi, j)
        qs = q_scrs[3 * (groups[gi][0] % 2) + j]
        return pltpu.bitcast(qs[pl.ds(zero(), T // 2), :GW], BF16)

    def k_operand(gi, i, w):
        if (gi, i, w) in fwd_k:
            return fwd_k.pop((gi, i, w))
        return pltpu.bitcast(k_scr[3 * i + w - 1][pl.ds(zero(), CR // 2), :], BF16)

    def finish(gi, i, w, ct, s):
        g, _, _, carry = groups[gi]
        s = s * c
        row = (w - 1) * (Sk // 2) + i * CR
        s_scrs[g % N_S][row:row + CR, ct * 128:ct * 128 + s.shape[1]] = s
        for n in range(s.shape[1] // 128):
            mx = run_max.get((gi, ct + n))
            for rr in range(CR // 8):
                x = s[rr * 8:(rr + 1) * 8, n * 128:(n + 1) * 128]
                mx = x if mx is None else jnp.maximum(mx, x)
            run_max[(gi, ct + n)] = mx
        tiles_done[gi] = tiles_done.get(gi, 0) + s.shape[1] // 128
        if tiles_done[gi] == (Sk // CR) * (GW // 128):
            mx = jnp.concatenate([run_max[(gi, n)] for n in range(GW // 128)], axis=1)
            m = jnp.broadcast_to(jnp.max(mx, axis=0, keepdims=True), (8, GW))
            if carry:
                m_scr[g * 8:(g + 1) * 8, :] = m
            else:
                m_fin[g] = m

    def qk_split(gi, i, head):
        qv = [q_third(gi, j) for j in q_parts[3]]
        kk = k_operand(gi, i, 3)
        for ct in range(GW // 128):
            lo, hi = (CR - STAGGER[ct], CR) if head else (0, CR - STAGGER[ct])
            wt = jnp.concatenate([x[:, ct * 128:(ct + 1) * 128] for x in qv], axis=0)
            p3_wide[lo:hi, ct * 128:(ct + 1) * 128] = jnp.dot(kk[lo:hi], wt,
                                                              preferred_element_type=F32)

    def qk_pass(gi, i, w):
        wt = jnp.concatenate([q_third(gi, j) for j in q_parts[w]], axis=0)
        pw = jnp.dot(k_operand(gi, i, w), wt, preferred_element_type=F32)
        results.append((starts[-1], CR, pw))
        finish(gi, i, w, 0, pw + p3_wide[pl.ds(zero(), CR), :GW])

    def qk_round(gi, i, rnd):
        qv = [q_third(gi, j) for j in range(3)]
        if groups[gi][2] is not None and rnd == 0 and (carried or i >= K_EARLY):
            prep_k(gi, i)
        kk = {w: k_operand(gi, i, w) for w in (1, 2, 3)}

        def dot(w, ct):
            wt = jnp.concatenate([qv[j][:, ct * 128:(ct + 1) * 128] for j in q_parts[w]], axis=0)
            return jnp.dot(kk[w], wt, preferred_element_type=F32)

        p3 = dot(3, rnd)
        results.append((starts[-1], CR, p3))
        finish(gi, i, 1, rnd, dot(1, rnd) + p3)
        finish(gi, i, 2, rnd, dot(2, rnd) + p3)
        if rnd == 0:
            p3_scrs[i % N_P3][...] = dot(3, 3)
        else:
            finish(gi, i, rnd, 3, dot(rnd, 3) + p3_scrs[i % N_P3][pl.ds(zero(), CR), :])

    s_off = {}
    state = {}

    def a_operand(i, hf):
        tiles = []
        for kp in range(hf * R // 128, (hf + 1) * R // 128):
            def blk(r, kr):
                return vt_ref[r * Dh:(r + 1) * Dh, (2 * kp + kr) * 128:(2 * kp + kr + 1) * 128]

            def add(x, y):
                return (blk(*x).astype(F32) + blk(*y).astype(F32)).astype(BF16)

            def sub(x, y):
                return (blk(*x).astype(F32) - blk(*y).astype(F32)).astype(BF16)

            tiles.append({1: lambda: add((0, 0), (1, 1)), 2: lambda: add((1, 0), (1, 1)),
                          3: lambda: blk(0, 0), 4: lambda: blk(1, 1),
                          5: lambda: add((0, 0), (0, 1)), 6: lambda: sub((1, 0), (0, 0)),
                          7: lambda: sub((0, 1), (1, 1))}[i]())
        return jnp.concatenate(tiles, axis=1)

    def pv(g, u, i, hf):
        if g not in s_off:
            s_off[g] = zero()
            if g < AHEAD:
                m_fin[g] = m_scr[g * 8:(g + 1) * 8, :]
        st = state.setdefault((g, u), {})

        def pbuf(kr, cx):
            return p_scrs[(u * 4 + kr * 2 + cx) * NH + hf]

        def fresh(kr, cx):
            cs = slice((2 * u + cx) * 128, (2 * u + cx + 1) * 128)
            s = s_scrs[g % N_S][pl.ds(s_off[g] + kr * (Sk // 2) + hf * R, R), cs]
            p = jnp.exp2(s - rep(tie(m_fin[g][:, cs], a_tie), R))
            pbuf(kr, cx)[...] = p
            return p

        def load(kr, cx):
            return pbuf(kr, cx)[pl.ds(zero(), R), :]

        def eager_sum(cx, p):
            la = st.get(("l", cx), [None] * 4)
            for tt in range(R // 128):
                for ii in range(7, -1, -1):
                    rr = tt * 128 + ii * 16
                    v = p[rr:rr + 8] + p[rr + 8:rr + 16]
                    la[tt % 4] = v if la[tt % 4] is None else la[tt % 4] + v
            if hf + 1 == NH:
                la = [(la[0] + la[1]) + (la[2] + la[3])] + [None] * (N_SUM - 1)
            st[("l", cx)] = la

        def lazy_sum(kr, cx):
            x = load(kr, cx)
            la = st[("l", cx)]
            for rr in range(R // 8):
                v = x[rr * 8:(rr + 1) * 8]
                la[rr % N_SUM] = v if la[rr % N_SUM] is None else la[rr % N_SUM] + v

        def total(cx):
            l8 = functools.reduce(lambda a, b: a + b, st[("l", cx)])
            return jnp.broadcast_to(jnp.sum(l8, axis=0, keepdims=True), (8, 128))

        def cross(kx, ky):
            if "rho" not in st:
                lx = total(0)
                st["rx"] = 1.0 / lx
                st["ry"] = 1.0 / total(1)
                st["rho"] = lx * st["ry"]
            rho = tie(st["rho"], b_tie)
            return load(kx, 0) - rep(rho, R) * load(ky, 1)

        if i == 2:
            w = fresh(0, 0)
            eager_sum(0, w)
        elif i == 4:
            w = fresh(1, 0) - load(0, 0)
            lazy_sum(1, 0)
        elif i == 5:
            w = fresh(1, 1)
            eager_sum(1, w)
        elif i == 3:
            w = load(1, 1) - fresh(0, 1)
            lazy_sum(0, 1)
        else:
            w = cross(*{1: (0, 1), 6: (0, 0), 7: (1, 1)}[i])
        if (g, u) != (0, 0):
            av = pltpu.bitcast(a_scrs[(i - 1) * NH + hf][pl.ds(zero(), Dh // 2), :], BF16)
        else:
            av = a_operand(i, hf)
            a_scrs[(i - 1) * NH + hf][...] = pltpu.bitcast(av, U32)
        mi = jnp.dot(av, w.astype(BF16), preferred_element_type=F32)
        if hf > 0:
            mi = mi + st.pop(("part", i))
        results.append((starts[-1], Dh, mi))
        if hf + 1 < NH:
            st[("part", i)] = mi
            return
        col = g * GW + u * 256

        def out(r, cx, x, scale):
            ot_ref[r * Dh:(r + 1) * Dh, col + cx * 128:col + (cx + 1) * 128] = (
                x * rep(scale, Dh)).astype(ot_ref.dtype)
            hook("tile", (r * Dh, col + cx * 128))

        if i in a_order:
            r_scrs[u * 4 + i - 2][...] = mi
        elif i == 1:
            m2, m3, m4, m5 = (r_scrs[u * 4 + j][pl.ds(zero(), Dh), :] for j in range(4))
            out(1, 0, m2 + m4, st["rx"])
            out(0, 1, m5 - m3, st["ry"])
            st["c11"] = mi + (m4 + rep(st["rho"], Dh) * m5)
            st["c22"] = (m2 - rep(st["rho"], Dh) * m3) - mi
        elif i == 6:
            out(1, 1, st.pop("c22") - mi, st["rx"])
        else:
            out(0, 0, mi + st.pop("c11"), st["rx"])
        if i == B_ORDER[-1]:
            hook("out", col + 256)

    q_jobs = [(qk_round, *ch, rnd) for ch in chunks[1 if carried else 0:] for rnd in range(3)]
    if carried:
        qk_split(*chunks[0], True)
        q_jobs[3:3] = [(qk_pass, *chunks[0], 2), (qk_pass, *chunks[0], 1)]
    else:
        for i in range(K_EARLY):
            prep_k(0, i)
        fwd_k.clear()
        hook("start", None)
    pairs = [(g, u) for g in pv_groups for u in range(2)]
    a_jobs = [pr + (i, hf) for pr in pairs for i in a_order for hf in range(NH)]
    b_jobs = [pr + (i, hf) for pr in pairs for i in B_ORDER for hf in range(NH)]
    na, nb = len(a_order) * NH, len(B_ORDER) * NH
    qi = ai = bi = pos = t = 0
    while qi < len(q_jobs) or ai < len(a_jobs) or bi < len(b_jobs):
        tok = prefix[pos] if pos < len(prefix) else cycle[(pos - len(prefix)) % len(cycle)]
        pos += 1
        if tok == "Q" and qi < len(q_jobs):
            fn, *args = q_jobs[qi]
            g, _, _, carry = groups[args[0]]
            assert not (carry and a_jobs) or ai >= 2 * na * (g + 1)
            hook("qk", qi)
            starts.append(t)
            fn(*args)
            qi += 1
            t += CR
        elif tok == "A" and ai < len(a_jobs):
            assert ai // na - bi // nb < 2
            starts.append(t)
            pv(*a_jobs[ai])
            ai += 1
            t += Dh
        elif tok == "B" and bi < len(b_jobs) and ai >= min((bi // nb + 1) * na + 1, len(a_jobs)):
            starts.append(t)
            pv(*b_jobs[bi])
            bi += 1
            t += Dh
        else:
            continue
        hook("job", qi + ai + bi)
    if tail is not None:
        stage_q(tail[0], 0)
        qk_split(*tail, False)


def _kernel(q_hbm, k_hbm, v_hbm, o_hbm, in_buf, o_buf, sem_in, sem_pro, sem_out, m_scr, p3_wide,
            *scrs, c):
    H, D, Sq = q_hbm.shape
    Sk = k_hbm.shape[2]
    ng = Sq // GW
    nch = Sk // (2 * CR)
    k_scr, scrs = scrs[:3 * nch], scrs[3 * nch:]
    s_scrs, scrs = scrs[:N_S], scrs[N_S:]
    a_scrs, scrs = scrs[:7 * NH], scrs[7 * NH:]
    q_scrs, scrs = scrs[:6], scrs[6:]
    p3_scrs, scrs = scrs[:N_P3], scrs[N_P3:]
    r_scrs, p_scrs = scrs[:8], scrs[8:]
    pid = pl.program_id(0)
    qa = (AHEAD + 1) * GW

    def start_inputs(h, hn, slot):
        pltpu.make_async_copy(v_hbm.at[h], in_buf.at[slot, 0], sem_in).start()
        pltpu.make_async_copy(q_hbm.at[h, :, qa:], in_buf.at[slot, 1, :, qa:], sem_in).start()
        pltpu.make_async_copy(k_hbm.at[hn], in_buf.at[slot, 2], sem_in).start()
        pltpu.make_async_copy(q_hbm.at[hn, :, :qa], in_buf.at[slot, 1, :, :qa], sem_in).start()

    def wait_inputs(slot):
        pltpu.make_async_copy(in_buf.at[slot], in_buf.at[slot], sem_in).wait()

    common = dict(k_scr=k_scr, s_scrs=s_scrs, a_scrs=a_scrs, q_scrs=q_scrs, p3_scrs=p3_scrs,
                  p3_wide=p3_wide, r_scrs=r_scrs, p_scrs=p_scrs, m_scr=m_scr, c=c, D=D, Sk=Sk)

    @pl.when(pid == 0)
    def _():
        ks = K_FIRST * 2 * CR
        ke = K_EARLY * 2 * CR
        early = pltpu.make_async_copy(k_hbm.at[0, :, :ke], in_buf.at[1, 2, :, :ke], sem_pro.at[4])
        first = [pltpu.make_async_copy(k_hbm.at[0, :, ke:ks], in_buf.at[1, 2, :, ke:ks], sem_pro.at[0]),
                 pltpu.make_async_copy(q_hbm.at[0, :, :GW], in_buf.at[1, 1, :, :GW], sem_pro.at[1])]
        second = [pltpu.make_async_copy(k_hbm.at[0, :, ks:], in_buf.at[1, 2, :, ks:], sem_pro.at[2]),
                  pltpu.make_async_copy(q_hbm.at[0, :, GW:qa], in_buf.at[1, 1, :, GW:qa], sem_pro.at[3])]
        for cp in [early] + first + second:
            cp.start()
        start_inputs(0, 1, 0)
        early.wait()
        groups0 = [(g, in_buf.at[1, 1], in_buf.at[1, 2] if g == 0 else None, True)
                   for g in range(AHEAD + 1)]
        chunks0 = ([(g, i) for g in range(AHEAD) for i in range(K_FIRST)]
                   + [(g, i) for g in range(AHEAD) for i in range(K_FIRST, nch)])

        def hook0(kind, x):
            if kind == "start":
                for cp in first:
                    cp.wait()
            if kind == "qk" and x == 3 * K_FIRST:
                for cp in second:
                    cp.wait()

        _emit(chunks0, (AHEAD, 0), [], groups0, plan=("", "Q", (), 0, 0), carried=False, fwd=True,
              seed=pid, vt_ref=None, ot_ref=None, hook=hook0, **common)

        def body(h, carry):
            slot = lax.bitwise_and(h, 1)
            cur = in_buf.at[slot]
            wait_inputs(slot)

            def hook(kind, x):
                if kind == "job" and x == DMA_AT:
                    start_inputs(h + 1, jnp.minimum(h + 2, H - 1), 1 - slot)

            groups = ([(g, cur.at[1], None, False) for g in range(AHEAD, ng)]
                      + [(g, cur.at[1], cur.at[2] if g == 0 else None, True)
                         for g in range(AHEAD + 1)])
            chunks = [(gi, i) for gi in range(ng) for i in range(nch)]
            _emit(chunks, (ng, 0), list(range(ng)), groups, plan=MAIN_PLAN, carried=True,
                  fwd=False, seed=h, vt_ref=cur.at[0], ot_ref=o_buf.at[h], hook=hook,
                  **common)
            pltpu.make_async_copy(o_buf.at[h], o_hbm.at[h], sem_out).start()
            return carry

        lax.fori_loop(0, H - 1, body, 0)

    @pl.when(pid == 1)
    def _():
        slot = (H - 1) % 2
        wait_inputs(slot)
        edges = [0, *LAST_EDGES]

        def hook(kind, x):
            if kind == "out" and x in edges[1:]:
                idx = (H - 1, slice(None), slice(edges[edges.index(x) - 1], x))
            elif kind == "tile" and x[1] >= edges[-1]:
                idx = (H - 1, slice(x[0], x[0] + D // 2), slice(x[1], x[1] + 128))
            else:
                return
            pltpu.make_async_copy(o_buf.at[idx], o_hbm.at[idx], sem_out).start()

        groups = [(g, in_buf.at[slot, 1], None, False) for g in range(AHEAD, ng)]
        chunks = [(gi, i) for gi in range(ng - AHEAD) for i in range(nch)]
        _emit(chunks, None, list(range(ng)), groups, plan=LAST_PLAN, carried=True, fwd=False,
              seed=pid, vt_ref=in_buf.at[slot, 0], ot_ref=o_buf.at[H - 1], hook=hook,
              **common)
        pltpu.make_async_copy(o_buf, o_hbm, sem_out).wait()


@jax.jit
def pallas_standalone__mha_softmax__prompt_kernel(
    q: jax.Array,
    k: jax.Array,
    v: jax.Array,
):
    B, H, Sq, D = q.shape
    Sk = k.shape[2]
    BH = B * H
    assert D == 192 and Sq == Sk == N_S * GW and BH >= 2
    c = D ** -0.5 * math.log2(math.e)
    R = Sk // 2 // NH
    qt, kt, vt = (jnp.swapaxes(x, 2, 3).reshape(BH, D, Sq) for x in (q, k, v))
    scratch = (
        [pltpu.VMEM((2, 3, D, Sq), BF16),
         pltpu.VMEM((BH, D, Sq), BF16),
         pltpu.SemaphoreType.DMA(()),
         pltpu.SemaphoreType.DMA((5,)),
         pltpu.SemaphoreType.DMA(()),
         pltpu.VMEM((AHEAD * 8, GW), F32),
         pltpu.VMEM((CR, GW + PAD), F32)]
        + [pltpu.VMEM((CR // 2, 2 * D // 3), U32)] * (3 * Sk // (2 * CR))
        + [pltpu.VMEM((Sk, GW + PAD), F32)] * N_S
        + [pltpu.VMEM((D // 4, R), U32)] * (7 * NH)
        + [pltpu.VMEM((D // 6, GW + PAD), U32)] * 6
        + [pltpu.VMEM((CR, 128), F32)] * N_P3
        + [pltpu.VMEM((D // 2, 128), F32)] * 8
        + [pltpu.VMEM((R, 128), F32)] * (8 * NH)
    )
    ot = pl.pallas_call(
        functools.partial(_kernel, c=c),
        grid=(2,),
        in_specs=[pl.BlockSpec(memory_space=pl.ANY)] * 3,
        out_specs=pl.BlockSpec(memory_space=pl.ANY),
        out_shape=jax.ShapeDtypeStruct((BH, D, Sq), q.dtype),
        scratch_shapes=scratch,
        compiler_params=pltpu.CompilerParams(
            dimension_semantics=("arbitrary",),
            vmem_limit_bytes=100 * 1024 * 1024,
            disable_bounds_checks=True,
        ),
    )(qt, kt, vt)
    return jnp.swapaxes(ot.reshape(B, H, D, Sq), 2, 3)
```
